```python
import jax
import jax.numpy as jnp

def _softmax(x, axis=-1):
    return jax.nn.softmax(x, axis=axis)

def _gelu(x):
    return jax.nn.gelu(x, approximate=True)

def _silu(x):
    return jax.nn.silu(x)

def _sigmoid(x):
    return jax.nn.sigmoid(x)

def _layernorm(x, axis=-1, eps=1e-05):
    m = jnp.mean(x, axis=axis, keepdims=True)
    v = jnp.var(x, axis=axis, keepdims=True)
    return (x - m) / jnp.sqrt(v + eps)

def _scatter_add(tgt, idx, src, axis=0):
    return tgt.at[idx].add(src)

def _segment_sum(src, seg, n):
    return jax.ops.segment_sum(src, seg, n)

class _Rng:

    def __init__(self, key):
        self._k = key

    def _next(self):
        self._k, sub = jax.random.split(self._k)
        return sub

    def normal(self, shape):
        return jax.random.normal(self._next(), shape, dtype=jnp.bfloat16)

    def randint(self, lo, hi, shape):
        return jax.random.randint(self._next(), shape, lo, hi, dtype=jnp.int32)

    def uniform(self, shape, lo=0.0, hi=1.0):
        return jax.random.uniform(self._next(), shape, jnp.bfloat16, lo, hi)

    def permutation(self, n):
        return jax.random.permutation(self._next(), n)
kernel_name = 'gated_mix__ssm_conv_h3__memory_aug_recurrent_mem_tr__prompt'

def setup_inputs():
    _rng = _Rng(jax.random.key(int.from_bytes(__import__("os").urandom(4), "little")))
    _w = lambda a: (lambda t: t.astype(jnp.bfloat16) if jnp.issubdtype(t.dtype, jnp.floating) else t)(jnp.asarray(a))

    def _A_setup():
        B, S, D = (1, 2048, 1024)
        ks = 4
        return {'q': _w((lambda *s: _rng.normal(s) * 0.05)(B, S, D)), 'k': _w((lambda *s: _rng.normal(s) * 0.05)(B, S, D)), 'v': _w((lambda *s: _rng.normal(s) * 0.05)(B, S, D)), 'shift_k': _w((lambda *s: _rng.normal(s) * 0.05)(D, ks) * 0.5), 'ssm_k': _w((lambda *s: _rng.normal(s) * 0.05)(D, S) * (1.0 / S ** 0.5)), 'ssm_D': _w((lambda *s: _rng.normal(s) * 0.05)(D))}
    _A_in = _A_setup()

    def _B_setup():
        B, S, Dm = (1, 2048, 1024)
        H, Dh = (32, 128)
        M, seg = (8, 32)
        seg = min(seg, S)
        S = S // seg * seg
        return {'x': _w((lambda *s: _rng.normal(s) * 0.05)(B, S, Dm)), 'mem0': _w((lambda *s: _rng.normal(s) * 0.05)(B, M, Dm)), 'Wq': _w((lambda *s: _rng.normal(s) * 0.05)(Dm, H, Dh) * Dm ** (-0.5)), 'Wk': _w((lambda *s: _rng.normal(s) * 0.05)(Dm, H, Dh) * Dm ** (-0.5)), 'Wv': _w((lambda *s: _rng.normal(s) * 0.05)(Dm, H, Dh) * Dm ** (-0.5)), 'Wo': _w((lambda *s: _rng.normal(s) * 0.05)(H, Dh, Dm) * (H * Dh) ** (-0.5)), 'seg_len': seg}
    _B_in = _B_setup()
    return {'A_q': _A_in['q'], 'A_k': _A_in['k'], 'A_v': _A_in['v'], 'A_shift_k': _A_in['shift_k'], 'A_ssm_k': _A_in['ssm_k'], 'A_ssm_D': _A_in['ssm_D'], 'B_x': _B_in['x'], 'B_mem0': _B_in['mem0'], 'B_Wq': _B_in['Wq'], 'B_Wk': _B_in['Wk'], 'B_Wv': _B_in['Wv'], 'B_Wo': _B_in['Wo'], 'B_seg_len': _B_in['seg_len'], 'gate_w': _w((lambda *s: _rng.normal(s) * 0.05)(1024))}

def reference(A_q, A_k, A_v, A_shift_k, A_ssm_k, A_ssm_D, B_x, B_mem0, B_Wq, B_Wk, B_Wv, B_Wo, B_seg_len, gate_w):

    def _A_ref(q, k, v, shift_k, ssm_k, ssm_D):
        B, S, D = q.shape
        ks = shift_k.shape[-1]
        k_pad = jnp.pad(k, ((0, 0), (ks - 1, 0), (0, 0)))
        k_shift = jnp.zeros_like(k)
        for t in range(ks):
            k_shift = k_shift + k_pad[:, t:t + S, :] * shift_k[:, ks - 1 - t][None, None, :]
        kv = k_shift * v
        L = 2 * S
        kv_pad = jnp.pad(kv, ((0, 0), (0, S), (0, 0)))
        kf_pad = jnp.pad(ssm_k, ((0, 0), (0, S)))
        kv_f = (lambda x, axes=(-2, -1): jnp.fft.rfft2(x.astype(jnp.float32), axes=axes))(kv_pad[:, None, :, :], axes=(1, 2))
        kf_f = (lambda x, axes=(-2, -1): jnp.fft.rfft2(x.astype(jnp.float32), axes=axes))(kf_pad[:, None, :], axes=(1, 2))
        kf_f = (lambda x, *d: x.transpose(*d))(kf_f, 1, 2, 0)
        y_f = kv_f * kf_f[None, :, :, :]
        y = (lambda x, s, axes=(-2, -1): jnp.fft.irfft2(x, s=s, axes=axes).astype(jnp.bfloat16))(y_f, (1, L), axes=(1, 2))[:, 0, :S, :]
        y = y + kv * ssm_D[None, None, :]
        return q * y

    def _B_ref(x, mem0, Wq, Wk, Wv, Wo, seg_len):
        B, S, Dm = x.shape
        H, Dh = (Wq.shape[1], Wq.shape[2])
        M = mem0.shape[1]
        scale = Dh ** (-0.5)
        n_seg = S // seg_len
        L = M + seg_len
        idx = jnp.arange(L)
        mask = (idx[:, None] < M) | (idx[:, None] >= idx[None, :])
        mem = mem0
        outs = []
        for s in range(n_seg):
            xs = x[:, s * seg_len:(s + 1) * seg_len, :].copy()
            h = jnp.concatenate([mem, xs], axis=1)
            q = jnp.einsum('btd,dhe->bhte', h, Wq)
            k = jnp.einsum('btd,dhe->bhte', h, Wk)
            v = jnp.einsum('btd,dhe->bhte', h, Wv)
            scores = jnp.einsum('bhqe,bhke->bhqk', q, k) * scale
            scores = jnp.where(mask[None, None], scores, -1000000000.0)
            p = _softmax(scores, axis=-1)
            o = jnp.einsum('bhqk,bhke->bhqe', p, v)
            o = jnp.einsum('bhte,hed->btd', o, Wo)
            mem = o[:, :M, :].copy()
            outs.append(o[:, M:, :])
        return jnp.concatenate(outs, axis=1)
    x = A_q
    g = _sigmoid((x * gate_w).sum(-1, keepdims=True))
    a = _A_ref(x, A_k, A_v, A_shift_k, A_ssm_k, A_ssm_D)
    b = _B_ref(x, B_mem0, B_Wq, B_Wk, B_Wv, B_Wo, B_seg_len)
    return g * a + (1 - g) * b
```

```python
import functools

import jax
import jax.numpy as jnp
import numpy as np
import jax.experimental.pallas as pl
import jax.experimental.pallas.tpu as pltpu

F32 = jnp.float32
BF16 = jnp.bfloat16
U32 = jnp.uint32

C = 128


def _dft_mats():
    f = np.arange(C, dtype=np.float64)[:, None] + 0.5
    t = np.arange(C, dtype=np.float64)[None, :]
    ang = 2.0 * np.pi * f * t / (2 * C)
    fwd = np.concatenate([np.cos(ang), -np.sin(ang)], axis=0)
    inv = np.concatenate([np.cos(ang).T, -np.sin(ang).T], axis=1) * (2.0 / (2 * C))
    return fwd.astype(np.float32), inv.astype(np.float32)


def _nt(a, b):
    return jax.lax.dot_general(a, b, (((1,), (1,)), ((), ())), preferred_element_type=F32)


def _nn(a, b):
    return jnp.dot(a, b, preferred_element_type=F32)


def _kernel(q_hbm, k_hbm, v_hbm, shift_ref, ssmk_hbm, ssmd_ref, mem0_ref,
            wq_hbm, wk_hbm, wv_hbm, wo_hbm, gate_ref, f_ref, fi_ref,
            out_hbm,
            qbuf, kbuf, vbuf, sbuf, raw, wqkv, wo, abuf, gbuf, obuf,
            taps, kvbuf, asp, ksp, ysp, membuf, pend, pendo, o32,
            sem_in, sem_q, sem_w, sem_wo, sem_out,
            *, S, D, H, seg, M):
    NG = D // 128
    NCH = S // C
    WCH = 4
    DCH = D // WCH

    def in_copies(g):
        sl = pl.ds(g * 128, 128)
        return (pltpu.make_async_copy(k_hbm.at[:, sl], kbuf.at[g], sem_in.at[0, g]),
                pltpu.make_async_copy(v_hbm.at[:, sl], vbuf.at[g], sem_in.at[1, g]),
                pltpu.make_async_copy(ssmk_hbm.at[sl, :], sbuf.at[g], sem_in.at[2, g]),
                pltpu.make_async_copy(q_hbm.at[:, sl], qbuf.at[g], sem_in.at[3, g]))

    def w_copy(i, c):
        src = (wq_hbm, wk_hbm, wv_hbm)[i]
        rows = pl.ds(c * DCH * H, DCH * H)
        return pltpu.make_async_copy(src.at[rows, :], raw.at[i, rows, :], sem_w.at[i, c])

    def wo_copy(n):
        return pltpu.make_async_copy(wo_hbm.at[:, pl.ds(n * 128, 128)], wo.at[n], sem_wo.at[n])

    for g in range(NG):
        for cp in in_copies(g):
            cp.start()
    for c in range(WCH):
        for i in range(3):
            w_copy(i, c).start()
    for n in range(NG):
        wo_copy(n).start()

    taps[...] = jnp.transpose(shift_ref[...].astype(F32))
    ks = shift_ref.shape[1]
    fmat = f_ref[...]
    sgn = 1.0 - 2.0 * (jax.lax.broadcasted_iota(jnp.int32, (8, 128), 0) % 2).astype(F32)

    def conv_group(g, _):
        for cp in in_copies(g):
            cp.wait()
        lanes = pl.ds(pl.multiple_of(g * 128, 128), 128)
        tp = taps[:, lanes]
        dvec = ssmd_ref[:, lanes].astype(F32)
        for j in range(NCH):
            cur = kbuf[g, j * C:(j + 1) * C, :].astype(F32)
            if j == 0:
                prev = jnp.zeros((16, 128), F32)
            else:
                prev = kbuf[g, j * C - 16:j * C, :].astype(F32)
            ext = jnp.concatenate([prev, cur], axis=0)
            acc = cur * tp[0:1, :]
            for u in range(1, ks):
                acc = acc + ext[16 - u:16 - u + C, :] * tp[u:u + 1, :]
            kv = (acc * vbuf[g, j * C:(j + 1) * C, :].astype(F32)).astype(BF16)
            kvbuf[j * C:(j + 1) * C, :] = kv
            asp[j] = _nn(fmat, kv)
            ksp[j] = _nt(fmat, sbuf[g, :, j * C:(j + 1) * C])

        def freq_block(fb, _):
            rr = pl.ds(pl.multiple_of(fb * 8, 8), 8)
            ri = pl.ds(pl.multiple_of(C + fb * 8, 8), 8)
            prev_z = None
            IB = 4
            for i0 in range(0, NCH, IB):
                kc = {}
                zr = [None] * IB
                zi = [None] * IB
                for j in range(i0 + IB):
                    ar, ai = asp[j, rr, :], asp[j, ri, :]
                    for ii in range(IB):
                        m = i0 + ii - j
                        if m < 0:
                            continue
                        if m not in kc:
                            kc[m] = (ksp[m, rr, :], ksp[m, ri, :])
                        kr, kim = kc[m]
                        pr = ar * kr - ai * kim
                        pi = ar * kim + ai * kr
                        zr[ii] = pr if zr[ii] is None else zr[ii] + pr
                        zi[ii] = pi if zi[ii] is None else zi[ii] + pi
                for ii in range(IB):
                    if prev_z is None:
                        yr, yi = zr[ii], zi[ii]
                    else:
                        yr = zr[ii] - sgn * prev_z[1]
                        yi = zi[ii] + sgn * prev_z[0]
                    prev_z = (zr[ii], zi[ii])
                    ysp[i0 + ii, rr, :] = yr
                    ysp[i0 + ii, ri, :] = yi
            return 0

        jax.lax.fori_loop(0, C // 8, freq_block, 0)

        fimat = fi_ref[...]
        for j in range(NCH):
            y = _nn(fimat, ysp[j].astype(BF16)).astype(BF16).astype(F32)
            kv = kvbuf[j * C:(j + 1) * C, :].astype(F32)
            y = (y + (kv * dvec).astype(BF16).astype(F32)).astype(BF16).astype(F32)
            qv = qbuf[g, j * C:(j + 1) * C, :].astype(F32)
            abuf[g, j * C:(j + 1) * C, :] = (qv * y).astype(BF16)
        return 0

    jax.lax.fori_loop(0, NG, conv_group, 0)

    gw = jnp.broadcast_to(gate_ref[...], (128, D))
    RB = 256

    def gate_blk(i, _):
        rows = pl.ds(pl.multiple_of(i * RB, RB), RB)
        x = jnp.concatenate([qbuf[g, rows, :] for g in range(NG)], axis=1)
        z = _nt(x, gw)
        gbuf[rows, :] = jax.nn.sigmoid(z)
        return 0

    jax.lax.fori_loop(0, S // RB, gate_blk, 0)

    HP = H // 2
    for c in range(WCH):
        for i in range(3):
            w_copy(i, c).wait()
            w32 = raw.at[i].bitcast(U32)

            def repack(b, _, i=i, c=c, w32=w32):
                d0 = c * DCH + b * 16
                blk = w32.at[pl.ds(pl.multiple_of(d0 * HP, 16 * HP), 16 * HP), :]
                dst = pl.ds(pl.multiple_of(d0 // 2, 8), 8)
                for hp in range(HP):
                    a = blk[pl.ds(hp, 8, stride=2 * HP), :]
                    b_ = blk[pl.ds(HP + hp, 8, stride=2 * HP), :]
                    wqkv[i * H + 2 * hp, dst, :] = (a & 0xFFFF) | (b_ << 16)
                    wqkv[i * H + 2 * hp + 1, dst, :] = (a >> 16) | (b_ & U32(0xFFFF0000))
                return 0

            jax.lax.fori_loop(0, DCH // 16, repack, 0)
    for n in range(NG):
        wo_copy(n).wait()

    membuf[...] = mem0_ref[...].astype(F32)
    L = M + seg
    scale = 128 ** -0.5
    row = jax.lax.broadcasted_iota(jnp.int32, (48, 48), 0)
    col = jax.lax.broadcasted_iota(jnp.int32, (48, 48), 1)
    mask = (col < L) & ((row < M) | (row >= col))

    def step(u, even):
        r0 = pl.multiple_of(u * 2 * seg, 2 * seg)
        if even:
            xs, nx = r0, 40
        else:
            xs, nx = r0 + 40, 24
        xs = pl.multiple_of(xs, 8)
        rows_m = M + nx
        lhs = jnp.concatenate(
            [jnp.concatenate([membuf[:, g * 128:(g + 1) * 128],
                              qbuf[g, pl.ds(xs, nx), :].astype(F32)], axis=0)
             for g in range(NG)], axis=1).astype(BF16)

        for h in range(H):
            prj = []
            for i in range(3):
                r = _nn(lhs, pltpu.bitcast(wqkv[i * H + h], BF16))
                if even:
                    pend[i * H + h] = r[40:48]
                    full = r
                else:
                    full = jnp.concatenate(
                        [r[0:8], pend[i * H + h], r[8:32], jnp.zeros((8, 128), F32)], axis=0)
                prj.append(full.astype(BF16))
            qh, kh, vh = prj
            s = _nt(qh, kh)
            s = jnp.where(mask, s, -1e9 / scale)
            mx = jnp.max(s, axis=1, keepdims=True)
            e = jnp.exp((s - mx) * scale)
            l = jnp.sum(e, axis=1, keepdims=True)
            o = _nn(e.astype(BF16), vh) * (1.0 / l)
            if even:
                pendo[h] = o[32:40]
                o32[h, 0:16, :] = pltpu.bitcast(o[0:32].astype(BF16), U32)
            else:
                oo = jnp.concatenate([o[0:8], pendo[h], o[8:40]], axis=0)
                o32[h] = pltpu.bitcast(oo.astype(BF16), U32)

        rows_o = 32 if even else 48
        nb = rows_o - M
        b0 = pl.multiple_of(r0 if even else r0 + 24, 8)
        brow = pl.ds(b0, nb)
        gv = gbuf[brow, :]
        for n in range(NG):
            ol = jnp.concatenate(
                [pltpu.bitcast(o32[h, 0:rows_o // 2, :], BF16) for h in range(H)], axis=1)
            r = _nn(ol, wo[n]).astype(BF16).astype(F32)
            membuf[:, n * 128:(n + 1) * 128] = r[0:M]
            b = r[M:]
            a = abuf[n, brow, :].astype(F32)
            obuf[brow, n * 128:(n + 1) * 128] = (b + gv * (a - b)).astype(BF16)

    def double_step(u, _):
        step(u, True)
        step(u, False)
        rows = pl.ds(pl.multiple_of(u * 2 * seg, 2 * seg), 2 * seg)
        pltpu.make_async_copy(obuf.at[rows, :], out_hbm.at[rows, :], sem_out).start()
        return 0

    jax.lax.fori_loop(0, S // (2 * seg), double_step, 0)
    pltpu.make_async_copy(obuf, out_hbm, sem_out).wait()


@functools.partial(jax.jit, static_argnames=("B_seg_len",))
def pallas_gated_mix__ssm_conv_h3__memory_aug_recurrent_mem_tr__prompt_kernel(
    A_q: jax.Array,
    A_k: jax.Array,
    A_v: jax.Array,
    A_shift_k: jax.Array,
    A_ssm_k: jax.Array,
    A_ssm_D: jax.Array,
    B_x: jax.Array,
    B_mem0: jax.Array,
    B_Wq: jax.Array,
    B_Wk: jax.Array,
    B_Wv: jax.Array,
    B_Wo: jax.Array,
    B_seg_len,
    gate_w: jax.Array,
):
    del B_x
    Bn, S, D = A_q.shape
    Dm, H, Dh = B_Wq.shape
    M = B_mem0.shape[1]
    seg = int(B_seg_len)
    assert Bn == 1 and Dh == 128 and Dm == D and M == 8 and seg == 32
    assert S % (2 * seg) == 0 and S % 256 == 0 and D % 512 == 0 and H % 2 == 0
    NG = D // 128
    fwd, inv = _dft_mats()

    any_spec = pl.BlockSpec(memory_space=pl.ANY)
    vmem_spec = pl.BlockSpec(memory_space=pltpu.VMEM)
    out = pl.pallas_call(
        functools.partial(_kernel, S=S, D=D, H=H, seg=seg, M=M),
        out_shape=jax.ShapeDtypeStruct((S, D), A_q.dtype),
        in_specs=[any_spec, any_spec, any_spec, vmem_spec, any_spec, vmem_spec, vmem_spec,
                  any_spec, any_spec, any_spec, any_spec, vmem_spec, vmem_spec, vmem_spec],
        out_specs=any_spec,
        scratch_shapes=[
            pltpu.VMEM((NG, S, 128), BF16),
            pltpu.VMEM((NG, S, 128), BF16),
            pltpu.VMEM((NG, S, 128), BF16),
            pltpu.VMEM((NG, 128, S), BF16),
            pltpu.VMEM((3, D * H, 128), BF16),
            pltpu.VMEM((3 * H, D // 2, 128), U32),
            pltpu.VMEM((NG, H * Dh, 128), BF16),
            pltpu.VMEM((NG, S, 128), BF16),
            pltpu.VMEM((S, 128), F32),
            pltpu.VMEM((S, D), BF16),
            pltpu.VMEM((A_shift_k.shape[1], D), F32),
            pltpu.VMEM((S, 128), BF16),
            pltpu.VMEM((S // C, 2 * C, 128), F32),
            pltpu.VMEM((S // C, 2 * C, 128), F32),
            pltpu.VMEM((S // C, 2 * C, 128), F32),
            pltpu.VMEM((M, D), F32),
            pltpu.VMEM((3 * H, 8, 128), F32),
            pltpu.VMEM((H, 8, 128), F32),
            pltpu.VMEM((H, 24, 128), U32),
            pltpu.SemaphoreType.DMA((4, NG)),
            pltpu.SemaphoreType.DMA((NG,)),
            pltpu.SemaphoreType.DMA((3, 4)),
            pltpu.SemaphoreType.DMA((NG,)),
            pltpu.SemaphoreType.DMA(()),
        ],
        compiler_params=pltpu.CompilerParams(vmem_limit_bytes=120 * 1024 * 1024),
    )(
        A_q.reshape(S, D), A_k.reshape(S, D), A_v.reshape(S, D), A_shift_k, A_ssm_k,
        A_ssm_D.reshape(1, D), B_mem0.reshape(M, D),
        B_Wq.reshape(D * H, Dh), B_Wk.reshape(D * H, Dh), B_Wv.reshape(D * H, Dh),
        B_Wo.reshape(H * Dh, D), gate_w.reshape(1, D),
        jnp.asarray(fwd, BF16), jnp.asarray(inv, BF16),
    )
    return out.reshape(Bn, S, D)
```

```python
import functools

import jax
import jax.numpy as jnp
import numpy as np
import jax.experimental.pallas as pl
import jax.experimental.pallas.tpu as pltpu

F32 = jnp.float32
BF16 = jnp.bfloat16
U32 = jnp.uint32

C = 128


def _dft_mats():
    f = np.arange(C, dtype=np.float64)[:, None] + 0.5
    t = np.arange(C, dtype=np.float64)[None, :]
    ang = 2.0 * np.pi * f * t / (2 * C)
    fwd = np.concatenate([np.cos(ang), -np.sin(ang)], axis=0)
    inv = np.concatenate([np.cos(ang).T, -np.sin(ang).T], axis=1) * (2.0 / (2 * C))
    return fwd.astype(np.float32), inv.astype(np.float32)


def _nt(a, b):
    return jax.lax.dot_general(a, b, (((1,), (1,)), ((), ())), preferred_element_type=F32)


def _nn(a, b):
    return jnp.dot(a, b, preferred_element_type=F32)


def _kernel(q_hbm, k_hbm, v_hbm, shift_ref, ssmk_hbm, ssmd_ref, mem0_ref,
            wq_hbm, wk_hbm, wv_hbm, wo_hbm, gate_ref, f_ref, fi_ref,
            out_hbm,
            qbuf, kbuf, vbuf, sbuf, raw, wqkv, wo, abuf, gbuf, obuf,
            kvbuf, asp, ksp, ysp, membuf, pend, pendo, o32, pacc,
            sem_in, sem_w, sem_wo, sem_out,
            *, S, D, H, seg, M):
    NG = D // 128
    NCH = S // C
    WCH = 4
    DCH = D // WCH

    def in_copies(g):
        sl = pl.ds(g * 128, 128)
        return (pltpu.make_async_copy(k_hbm.at[:, sl], kbuf.at[g], sem_in.at[0, g]),
                pltpu.make_async_copy(v_hbm.at[:, sl], vbuf.at[g], sem_in.at[1, g]),
                pltpu.make_async_copy(ssmk_hbm.at[sl, :], sbuf.at[g], sem_in.at[2, g]),
                pltpu.make_async_copy(q_hbm.at[:, sl], qbuf.at[g], sem_in.at[3, g]))

    def w_copy(i, c):
        src = (wq_hbm, wk_hbm, wv_hbm)[i]
        rows = pl.ds(c * DCH * H, DCH * H)
        return pltpu.make_async_copy(src.at[rows, :], raw.at[i, rows, :], sem_w.at[i, c])

    def wo_copy(n):
        return pltpu.make_async_copy(wo_hbm.at[:, pl.ds(n * 128, 128)], wo.at[n], sem_wo.at[n])

    for g in range(NG):
        for cp in in_copies(g):
            cp.start()
    for c in range(WCH):
        for i in range(3):
            w_copy(i, c).start()
    for n in range(NG):
        wo_copy(n).start()

    ks = shift_ref.shape[0]
    fmat = f_ref[...]
    sgn = 1.0 - 2.0 * (jax.lax.broadcasted_iota(jnp.int32, (8, 128), 0) % 2).astype(F32)

    def conv_group(g, _):
        for cp in in_copies(g):
            cp.wait()
        lanes = pl.ds(pl.multiple_of(g * 128, 128), 128)
        tp = shift_ref[:, lanes].astype(F32)
        dvec = ssmd_ref[:, lanes].astype(F32)
        for j in range(NCH):
            cur = kbuf[g, j * C:(j + 1) * C, :].astype(F32)
            if j == 0:
                prev = jnp.zeros((16, 128), F32)
            else:
                prev = kbuf[g, j * C - 16:j * C, :].astype(F32)
            ext = jnp.concatenate([prev, cur], axis=0)
            acc = cur * tp[0:1, :]
            for u in range(1, ks):
                acc = acc + ext[16 - u:16 - u + C, :] * tp[u:u + 1, :]
            kv = (acc * vbuf[g, j * C:(j + 1) * C, :].astype(F32)).astype(BF16)
            kvbuf[j * C:(j + 1) * C, :] = kv
            asp[j] = _nn(fmat, kv)
            ksp[j] = _nt(fmat, sbuf[g, :, j * C:(j + 1) * C])

        def freq_block(fb, _):
            rr = pl.ds(pl.multiple_of(fb * 8, 8), 8)
            ri = pl.ds(pl.multiple_of(C + fb * 8, 8), 8)
            prev_z = None
            IB = 4
            for i0 in range(0, NCH, IB):
                kc = {}
                zr = [None] * IB
                zi = [None] * IB
                for j in range(i0 + IB):
                    ar, ai = asp[j, rr, :], asp[j, ri, :]
                    for ii in range(IB):
                        m = i0 + ii - j
                        if m < 0:
                            continue
                        if m not in kc:
                            kc[m] = (ksp[m, rr, :], ksp[m, ri, :])
                        kr, kim = kc[m]
                        pr = ar * kr - ai * kim
                        pi = ar * kim + ai * kr
                        zr[ii] = pr if zr[ii] is None else zr[ii] + pr
                        zi[ii] = pi if zi[ii] is None else zi[ii] + pi
                for ii in range(IB):
                    if prev_z is None:
                        yr, yi = zr[ii], zi[ii]
                    else:
                        yr = zr[ii] - sgn * prev_z[1]
                        yi = zi[ii] + sgn * prev_z[0]
                    prev_z = (zr[ii], zi[ii])
                    ysp[i0 + ii, rr, :] = yr
                    ysp[i0 + ii, ri, :] = yi
            return 0

        jax.lax.fori_loop(0, C // 8, freq_block, 0)

        fimat = fi_ref[...]
        for j in range(NCH):
            y = _nn(fimat, ysp[j].astype(BF16)).astype(BF16).astype(F32)
            kv = kvbuf[j * C:(j + 1) * C, :].astype(F32)
            y = (y + (kv * dvec).astype(BF16).astype(F32)).astype(BF16).astype(F32)
            qv = qbuf[g, j * C:(j + 1) * C, :].astype(F32)
            abuf[g, j * C:(j + 1) * C, :] = (qv * y).astype(BF16)
        return 0

    jax.lax.fori_loop(0, NG, conv_group, 0)

    gw = jnp.broadcast_to(gate_ref[...], (128, D))
    RB = 256

    def gate_blk(i, _):
        rows = pl.ds(pl.multiple_of(i * RB, RB), RB)
        x = jnp.concatenate([qbuf[g, rows, :] for g in range(NG)], axis=1)
        z = _nt(x, gw)
        gbuf[rows, :] = jax.nn.sigmoid(z)
        return 0

    jax.lax.fori_loop(0, S // RB, gate_blk, 0)

    HP = H // 2
    for c in range(WCH):
        for i in range(3):
            w_copy(i, c).wait()
            w32 = raw.at[i].bitcast(U32)

            def repack(b, _, i=i, c=c, w32=w32):
                d0 = c * DCH + b * 16
                blk = w32.at[pl.ds(pl.multiple_of(d0 * HP, 16 * HP), 16 * HP), :]
                dst = pl.ds(pl.multiple_of(d0 // 2, 8), 8)
                for hp in range(HP):
                    a = blk[pl.ds(hp, 8, stride=2 * HP), :]
                    b_ = blk[pl.ds(HP + hp, 8, stride=2 * HP), :]
                    wqkv[i * H + 2 * hp, dst, :] = (a & 0xFFFF) | (b_ << 16)
                    wqkv[i * H + 2 * hp + 1, dst, :] = (a >> 16) | (b_ & U32(0xFFFF0000))
                return 0

            jax.lax.fori_loop(0, DCH // 16, repack, 0)
    for n in range(NG):
        wo_copy(n).wait()

    membuf[...] = mem0_ref[...].astype(F32)
    L = M + seg
    scale = 128 ** -0.5
    row = jax.lax.broadcasted_iota(jnp.int32, (L, 48), 0)
    col = jax.lax.broadcasted_iota(jnp.int32, (L, 48), 1)
    mask = (col < L) & ((row < M) | (row >= col))

    def step(u, even):
        r0 = pl.multiple_of(u * 2 * seg, 2 * seg)
        if even:
            xs, nx = r0, 40
        else:
            xs, nx = r0 + 40, 24
        xs = pl.multiple_of(xs, 8)
        rows_m = M + nx
        lhs = jnp.concatenate(
            [jnp.concatenate([membuf[:, g * 128:(g + 1) * 128],
                              qbuf[g, pl.ds(xs, nx), :].astype(F32)], axis=0)
             for g in range(NG)], axis=1).astype(BF16)

        rows_o = 32 if even else 48
        nb = rows_o - M
        b0 = pl.multiple_of(r0 if even else r0 + 24, 8)
        brow = pl.ds(b0, nb)
        qkv, es = {}, {}

        def proj(h):
            res = []
            for i in range(3):
                r = _nn(lhs, pltpu.bitcast(wqkv[i * H + h], BF16))
                if even:
                    pend[i * H + h] = r[40:48]
                    full = r
                else:
                    full = jnp.concatenate(
                        [r[0:8], pend[i * H + h], r[8:32], jnp.zeros((8, 128), F32)], axis=0)
                res.append(full.astype(BF16))
            qkv[h] = res

        def scores(h):
            qh, kh, _ = qkv[h]
            s = _nt(qh, kh)[:L]
            s = jnp.where(mask, s, -1e9 / scale)
            mx = jnp.max(s, axis=1, keepdims=True)
            e = jnp.exp((s - mx) * scale)
            l = jnp.sum(e, axis=1, keepdims=True)
            e = jnp.concatenate([e, jnp.zeros((48 - L, 48), F32)], axis=0).astype(BF16)
            es[h] = (e, 1.0 / l)

        def attend(h):
            e, rl = es.pop(h)
            o = _nn(e, qkv.pop(h)[2])[:L] * rl
            if even:
                pendo[h] = o[32:40]
                o32[h, 0:16, :] = pltpu.bitcast(o[0:32].astype(BF16), U32)
            else:
                oo = jnp.concatenate([o[0:8], pendo[h], o[8:40]], axis=0)
                o32[h] = pltpu.bitcast(oo.astype(BF16), U32)

        def out_proj(n, h0, h1):
            ol = jnp.concatenate(
                [pltpu.bitcast(o32[h, 0:rows_o // 2, :], BF16) for h in range(h0, h1)], axis=1)
            return _nn(ol, wo[n, h0 * 128:h1 * 128, :])

        LAG = 2
        HS = 8
        for t in range(H + 1 + LAG):
            if t < H:
                proj(t)
            if t == H:
                for n in range(NG):
                    pacc[0:rows_o, n * 128:(n + 1) * 128] = out_proj(n, 0, HS)
            if 0 <= t - 1 < H:
                scores(t - 1)
            if 0 <= t - 1 - LAG < H:
                attend(t - 1 - LAG)

        gv = gbuf[brow, :]
        for n in range(NG):
            r = out_proj(n, HS, H) + pacc[0:rows_o, n * 128:(n + 1) * 128]
            r = r.astype(BF16).astype(F32)
            membuf[:, n * 128:(n + 1) * 128] = r[0:M]
            b = r[M:]
            a = abuf[n, brow, :].astype(F32)
            obuf[brow, n * 128:(n + 1) * 128] = (b + gv * (a - b)).astype(BF16)

    def double_step(u, _):
        step(u, True)
        step(u, False)
        rows = pl.ds(pl.multiple_of(u * 2 * seg, 2 * seg), 2 * seg)
        pltpu.make_async_copy(obuf.at[rows, :], out_hbm.at[rows, :], sem_out).start()
        return 0

    jax.lax.fori_loop(0, S // (2 * seg), double_step, 0)
    pltpu.make_async_copy(obuf, out_hbm, sem_out).wait()


@functools.partial(jax.jit, static_argnames=("B_seg_len",))
def pallas_gated_mix__ssm_conv_h3__memory_aug_recurrent_mem_tr__prompt_kernel(
    A_q: jax.Array,
    A_k: jax.Array,
    A_v: jax.Array,
    A_shift_k: jax.Array,
    A_ssm_k: jax.Array,
    A_ssm_D: jax.Array,
    B_x: jax.Array,
    B_mem0: jax.Array,
    B_Wq: jax.Array,
    B_Wk: jax.Array,
    B_Wv: jax.Array,
    B_Wo: jax.Array,
    B_seg_len,
    gate_w: jax.Array,
):
    del B_x
    Bn, S, D = A_q.shape
    Dm, H, Dh = B_Wq.shape
    M = B_mem0.shape[1]
    seg = int(B_seg_len)
    assert Bn == 1 and Dh == 128 and Dm == D and M == 8 and seg == 32
    assert S % (2 * seg) == 0 and S % 256 == 0 and D % 512 == 0 and H % 2 == 0
    NG = D // 128
    fwd, inv = _dft_mats()

    any_spec = pl.BlockSpec(memory_space=pl.ANY)
    vmem_spec = pl.BlockSpec(memory_space=pltpu.VMEM)
    out = pl.pallas_call(
        functools.partial(_kernel, S=S, D=D, H=H, seg=seg, M=M),
        out_shape=jax.ShapeDtypeStruct((S, D), A_q.dtype),
        in_specs=[any_spec, any_spec, any_spec, vmem_spec, any_spec, vmem_spec, vmem_spec,
                  any_spec, any_spec, any_spec, any_spec, vmem_spec, vmem_spec, vmem_spec],
        out_specs=any_spec,
        scratch_shapes=[
            pltpu.VMEM((NG, S, 128), BF16),
            pltpu.VMEM((NG, S, 128), BF16),
            pltpu.VMEM((NG, S, 128), BF16),
            pltpu.VMEM((NG, 128, S), BF16),
            pltpu.VMEM((3, D * H, 128), BF16),
            pltpu.VMEM((3 * H, D // 2, 128), U32),
            pltpu.VMEM((NG, H * Dh, 128), BF16),
            pltpu.VMEM((NG, S, 128), BF16),
            pltpu.VMEM((S, 128), F32),
            pltpu.VMEM((S, D), BF16),
            pltpu.VMEM((S, 128), BF16),
            pltpu.VMEM((S // C, 2 * C, 128), F32),
            pltpu.VMEM((S // C, 2 * C, 128), F32),
            pltpu.VMEM((S // C, 2 * C, 128), F32),
            pltpu.VMEM((M, D), F32),
            pltpu.VMEM((3 * H, 8, 128), F32),
            pltpu.VMEM((H, 8, 128), F32),
            pltpu.VMEM((H, 24, 128), U32),
            pltpu.VMEM((48, D), F32),
            pltpu.SemaphoreType.DMA((4, NG)),
            pltpu.SemaphoreType.DMA((3, 4)),
            pltpu.SemaphoreType.DMA((NG,)),
            pltpu.SemaphoreType.DMA(()),
        ],
        compiler_params=pltpu.CompilerParams(vmem_limit_bytes=120 * 1024 * 1024),
    )(
        A_q.reshape(S, D), A_k.reshape(S, D), A_v.reshape(S, D), A_shift_k.T, A_ssm_k,
        A_ssm_D.reshape(1, D), B_mem0.reshape(M, D),
        B_Wq.reshape(D * H, Dh), B_Wk.reshape(D * H, Dh), B_Wv.reshape(D * H, Dh),
        B_Wo.reshape(H * Dh, D), gate_w.reshape(1, D),
        jnp.asarray(fwd, BF16), jnp.asarray(inv, BF16),
    )
    return out.reshape(Bn, S, D)
```

```python
import functools

import jax
import jax.numpy as jnp
import numpy as np
import jax.experimental.pallas as pl
import jax.experimental.pallas.tpu as pltpu

F32 = jnp.float32
BF16 = jnp.bfloat16
U32 = jnp.uint32

C = 128


def _dft_mats():
    f = np.arange(C, dtype=np.float64)[:, None] + 0.5
    t = np.arange(C, dtype=np.float64)[None, :]
    ang = 2.0 * np.pi * f * t / (2 * C)
    fwd = np.concatenate([np.cos(ang), -np.sin(ang)], axis=0)
    inv = np.concatenate([np.cos(ang).T, -np.sin(ang).T], axis=1) * (2.0 / (2 * C))
    return fwd.astype(np.float32), inv.astype(np.float32)


def _nt(a, b):
    return jax.lax.dot_general(a, b, (((1,), (1,)), ((), ())), preferred_element_type=F32)


def _nn(a, b):
    return jnp.dot(a, b, preferred_element_type=F32)


def _kernel(q_hbm, k_hbm, v_hbm, shift_ref, ssmk_hbm, ssmd_ref, mem0_ref,
            wq_hbm, wk_hbm, wv_hbm, wo_hbm, gate_ref, f_ref, fi_ref,
            out_hbm,
            qbuf, kbuf, vbuf, sbuf, raw, wqkv, wo, abuf, gbuf, obuf,
            dskip, kvbuf, asp, ksp, ysp, membuf, pend, pendo, o32, pacc,
            sem_in, sem_wo, sem_out,
            *, S, D, H, seg, M):
    NG = D // 128
    NCH = S // C
    DCH = D // NG
    HP = H // 2
    CR = DCH * HP

    def in_copies(g):
        sl = pl.ds(pl.multiple_of(g * 128, 128), 128)
        rows = pl.ds(pl.multiple_of(g * CR, CR), CR)
        cps = [pltpu.make_async_copy(k_hbm.at[:, sl], kbuf.at[g], sem_in.at[0, g]),
               pltpu.make_async_copy(v_hbm.at[:, sl], vbuf.at[g], sem_in.at[1, g]),
               pltpu.make_async_copy(ssmk_hbm.at[sl, :], sbuf.at[g], sem_in.at[2, g]),
               pltpu.make_async_copy(q_hbm.at[:, sl], qbuf.at[g], sem_in.at[3, g])]
        for i, w in enumerate((wq_hbm, wk_hbm, wv_hbm)):
            cps.append(pltpu.make_async_copy(
                w.bitcast(U32).at[rows, :], raw.at[i, g], sem_in.at[4 + i, g]))
        return cps

    def wo_copy(n):
        return pltpu.make_async_copy(wo_hbm.at[:, pl.ds(n * 128, 128)], wo.at[n], sem_wo.at[n])

    AHEAD = 2
    for g in range(AHEAD):
        for cp in in_copies(g):
            cp.start()

    ks = shift_ref.shape[0]
    dskip[...] = ssmd_ref[...].astype(F32).reshape(1, D)
    fmat = f_ref[...]
    sgn = 1.0 - 2.0 * (jax.lax.broadcasted_iota(jnp.int32, (8, 128), 0) % 2).astype(F32)

    def repack(g, i, b):
        x = raw[i, g, b * 16 * HP:(b + 1) * 16 * HP, :].reshape(8, 2, HP // 8, 8, 128)
        dst = pl.ds(pl.multiple_of(g * (DCH // 2) + b * 8, 8), 8)
        for t in range(HP // 8):
            ev = jnp.transpose(x[:, 0, t], (1, 0, 2))
            od = jnp.transpose(x[:, 1, t], (1, 0, 2))
            for j in range(8):
                h = i * H + 2 * (8 * t + j)
                wqkv[h, dst, :] = (ev[j] & 0xFFFF) | (od[j] << 16)
                wqkv[h + 1, dst, :] = (ev[j] >> 16) | (od[j] & U32(0xFFFF0000))

    def conv_group(g, _):
        for cp in in_copies(g):
            cp.wait()

        @pl.when(g + AHEAD < NG)
        def _():
            for cp in in_copies(g + AHEAD):
                cp.start()

        @pl.when(g + AHEAD == NG)
        def _():
            for n in range(NG):
                wo_copy(n).start()

        lanes = pl.ds(pl.multiple_of(g * 128, 128), 128)
        tp = shift_ref[:, lanes].astype(F32)
        dvec = dskip[:, lanes]
        for j in range(NCH):
            cur = kbuf[g, j * C:(j + 1) * C, :].astype(F32)
            if j == 0:
                prev = jnp.zeros((16, 128), F32)
            else:
                prev = kbuf[g, j * C - 16:j * C, :].astype(F32)
            ext = jnp.concatenate([prev, cur], axis=0)
            acc = cur * tp[0:1, :]
            for u in range(1, ks):
                acc = acc + ext[16 - u:16 - u + C, :] * tp[u:u + 1, :]
            kv = (acc * vbuf[g, j * C:(j + 1) * C, :].astype(F32)).astype(BF16)
            kvbuf[j * C:(j + 1) * C, :] = kv
            asp[j] = _nn(fmat, kv)
            ksp[j] = _nt(fmat, sbuf[g, :, j * C:(j + 1) * C])
            for bi in range(j * 3 * DCH // (16 * NCH), (j + 1) * 3 * DCH // (16 * NCH)):
                repack(g, bi // (DCH // 16), bi % (DCH // 16))

        def freq_block(fb, _):
            rr = pl.ds(pl.multiple_of(fb * 8, 8), 8)
            ri = pl.ds(pl.multiple_of(C + fb * 8, 8), 8)
            prev_z = None
            IB = 4
            for i0 in range(0, NCH, IB):
                kc = {}
                zr = [None] * IB
                zi = [None] * IB
                for j in range(i0 + IB):
                    ar, ai = asp[j, rr, :], asp[j, ri, :]
                    for ii in range(IB):
                        m = i0 + ii - j
                        if m < 0:
                            continue
                        if m not in kc:
                            kc[m] = (ksp[m, rr, :], ksp[m, ri, :])
                        kr, kim = kc[m]
                        pr = ar * kr - ai * kim
                        pi = ar * kim + ai * kr
                        zr[ii] = pr if zr[ii] is None else zr[ii] + pr
                        zi[ii] = pi if zi[ii] is None else zi[ii] + pi
                for ii in range(IB):
                    if prev_z is None:
                        yr, yi = zr[ii], zi[ii]
                    else:
                        yr = zr[ii] - sgn * prev_z[1]
                        yi = zi[ii] + sgn * prev_z[0]
                    prev_z = (zr[ii], zi[ii])
                    ysp[i0 + ii, rr, :] = yr
                    ysp[i0 + ii, ri, :] = yi
            return 0

        jax.lax.fori_loop(0, C // 8, freq_block, 0)

        fimat = fi_ref[...]
        for j in range(NCH):
            y = _nn(fimat, ysp[j].astype(BF16)).astype(BF16).astype(F32)
            kv = kvbuf[j * C:(j + 1) * C, :].astype(F32)
            y = (y + (kv * dvec).astype(BF16).astype(F32)).astype(BF16).astype(F32)
            qv = qbuf[g, j * C:(j + 1) * C, :].astype(F32)
            abuf[g, j * C:(j + 1) * C, :] = (qv * y).astype(BF16)
        return 0

    jax.lax.fori_loop(0, NG, conv_group, 0)

    gw = jnp.broadcast_to(gate_ref[...].reshape(1, D), (128, D))
    RB = 256

    def gate_blk(i, _):
        rows = pl.ds(pl.multiple_of(i * RB, RB), RB)
        x = jnp.concatenate([qbuf[g, rows, :] for g in range(NG)], axis=1)
        z = _nt(x, gw)
        gbuf[rows, :] = jax.nn.sigmoid(z)
        return 0

    jax.lax.fori_loop(0, S // RB, gate_blk, 0)

    for n in range(NG):
        wo_copy(n).wait()

    membuf[...] = mem0_ref[...].astype(F32)
    L = M + seg
    scale = 128 ** -0.5
    row = jax.lax.broadcasted_iota(jnp.int32, (L, 48), 0)
    col = jax.lax.broadcasted_iota(jnp.int32, (L, 48), 1)
    mask = (col < L) & ((row < M) | (row >= col))

    def step(u, even):
        r0 = pl.multiple_of(u * 2 * seg, 2 * seg)
        if even:
            xs, nx = r0, 40
        else:
            xs, nx = r0 + 40, 24
        xs = pl.multiple_of(xs, 8)
        rows_m = M + nx
        lhs = jnp.concatenate(
            [jnp.concatenate([membuf[:, g * 128:(g + 1) * 128],
                              qbuf[g, pl.ds(xs, nx), :].astype(F32)], axis=0)
             for g in range(NG)], axis=1).astype(BF16)

        rows_o = 32 if even else 48
        nb = rows_o - M
        b0 = pl.multiple_of(r0 if even else r0 + 24, 8)
        brow = pl.ds(b0, nb)
        qkv, es = {}, {}

        def proj(h):
            res = []
            for i in range(3):
                r = _nn(lhs, pltpu.bitcast(wqkv[i * H + h], BF16))
                if even:
                    pend[i * H + h] = r[40:48]
                    full = r
                else:
                    full = jnp.concatenate(
                        [r[0:8], pend[i * H + h], r[8:32], jnp.zeros((8, 128), F32)], axis=0)
                res.append(full.astype(BF16))
            qkv[h] = res

        def scores(h):
            qh, kh, _ = qkv[h]
            s = _nt(qh, kh)[:L]
            s = jnp.where(mask, s, -1e9 / scale)
            mx = jnp.max(s, axis=1, keepdims=True)
            e = jnp.exp((s - mx) * scale)
            l = jnp.sum(e, axis=1, keepdims=True)
            e = jnp.concatenate([e, jnp.zeros((48 - L, 48), F32)], axis=0).astype(BF16)
            es[h] = (e, 1.0 / l)

        def attend(h):
            e, rl = es.pop(h)
            o = _nn(e, qkv.pop(h)[2])[:L] * rl
            if even:
                pendo[h] = o[32:40]
                o32[h, 0:16, :] = pltpu.bitcast(o[0:32].astype(BF16), U32)
            else:
                oo = jnp.concatenate([o[0:8], pendo[h], o[8:40]], axis=0)
                o32[h] = pltpu.bitcast(oo.astype(BF16), U32)

        def out_proj(n, h0, h1):
            ol = jnp.concatenate(
                [pltpu.bitcast(o32[h, 0:rows_o // 2, :], BF16) for h in range(h0, h1)], axis=1)
            return _nn(ol, wo[n, h0 * 128:h1 * 128, :])

        LAG = 2
        HS = 8
        for t in range(H + 1 + LAG):
            if t < H:
                proj(t)
            if t == H:
                for n in range(NG):
                    pacc[0:rows_o, n * 128:(n + 1) * 128] = out_proj(n, 0, HS)
            if 0 <= t - 1 < H:
                scores(t - 1)
            if 0 <= t - 1 - LAG < H:
                attend(t - 1 - LAG)

        gv = gbuf[brow, :]
        for n in range(NG):
            r = out_proj(n, HS, H) + pacc[0:rows_o, n * 128:(n + 1) * 128]
            r = r.astype(BF16).astype(F32)
            membuf[:, n * 128:(n + 1) * 128] = r[0:M]
            b = r[M:]
            a = abuf[n, brow, :].astype(F32)
            obuf[brow, n * 128:(n + 1) * 128] = (b + gv * (a - b)).astype(BF16)

    def double_step(u, _):
        step(u, True)
        step(u, False)
        rows = pl.ds(pl.multiple_of(u * 2 * seg, 2 * seg), 2 * seg)
        pltpu.make_async_copy(obuf.at[rows, :], out_hbm.at[rows, :], sem_out).start()
        return 0

    jax.lax.fori_loop(0, S // (2 * seg), double_step, 0)
    pltpu.make_async_copy(obuf, out_hbm, sem_out).wait()


@functools.partial(jax.jit, static_argnames=("B_seg_len",))
def pallas_gated_mix__ssm_conv_h3__memory_aug_recurrent_mem_tr__prompt_kernel(
    A_q: jax.Array,
    A_k: jax.Array,
    A_v: jax.Array,
    A_shift_k: jax.Array,
    A_ssm_k: jax.Array,
    A_ssm_D: jax.Array,
    B_x: jax.Array,
    B_mem0: jax.Array,
    B_Wq: jax.Array,
    B_Wk: jax.Array,
    B_Wv: jax.Array,
    B_Wo: jax.Array,
    B_seg_len,
    gate_w: jax.Array,
):
    del B_x
    Bn, S, D = A_q.shape
    Dm, H, Dh = B_Wq.shape
    M = B_mem0.shape[1]
    seg = int(B_seg_len)
    assert Bn == 1 and Dh == 128 and Dm == D and M == 8 and seg == 32
    assert S % (2 * seg) == 0 and S % 256 == 0 and D % 128 == 0 and D // 128 >= 2 and H % 16 == 0
    NG = D // 128
    fwd, inv = _dft_mats()

    any_spec = pl.BlockSpec(memory_space=pl.ANY)
    vmem_spec = pl.BlockSpec(memory_space=pltpu.VMEM)
    out = pl.pallas_call(
        functools.partial(_kernel, S=S, D=D, H=H, seg=seg, M=M),
        out_shape=jax.ShapeDtypeStruct((S, D), A_q.dtype),
        in_specs=[any_spec, any_spec, any_spec, vmem_spec, any_spec, vmem_spec, vmem_spec,
                  any_spec, any_spec, any_spec, any_spec, vmem_spec, vmem_spec, vmem_spec],
        out_specs=any_spec,
        scratch_shapes=[
            pltpu.VMEM((NG, S, 128), BF16),
            pltpu.VMEM((NG, S, 128), BF16),
            pltpu.VMEM((NG, S, 128), BF16),
            pltpu.VMEM((NG, 128, S), BF16),
            pltpu.VMEM((3, NG, D * H // (2 * NG), 128), U32),
            pltpu.VMEM((3 * H, D // 2, 128), U32),
            pltpu.VMEM((NG, H * Dh, 128), BF16),
            pltpu.VMEM((NG, S, 128), BF16),
            pltpu.VMEM((S, 128), F32),
            pltpu.VMEM((S, D), BF16),
            pltpu.VMEM((1, D), F32),
            pltpu.VMEM((S, 128), BF16),
            pltpu.VMEM((S // C, 2 * C, 128), F32),
            pltpu.VMEM((S // C, 2 * C, 128), F32),
            pltpu.VMEM((S // C, 2 * C, 128), F32),
            pltpu.VMEM((M, D), F32),
            pltpu.VMEM((3 * H, 8, 128), F32),
            pltpu.VMEM((H, 8, 128), F32),
            pltpu.VMEM((H, 24, 128), U32),
            pltpu.VMEM((48, D), F32),
            pltpu.SemaphoreType.DMA((7, NG)),
            pltpu.SemaphoreType.DMA((NG,)),
            pltpu.SemaphoreType.DMA(()),
        ],
        compiler_params=pltpu.CompilerParams(vmem_limit_bytes=120 * 1024 * 1024),
    )(
        A_q.reshape(S, D), A_k.reshape(S, D), A_v.reshape(S, D), A_shift_k.T, A_ssm_k,
        A_ssm_D, B_mem0.reshape(M, D),
        B_Wq.reshape(D * H, Dh), B_Wk.reshape(D * H, Dh), B_Wv.reshape(D * H, Dh),
        B_Wo.reshape(H * Dh, D), gate_w,
        jnp.asarray(fwd, BF16), jnp.asarray(inv, BF16),
    )
    return out.reshape(Bn, S, D)
```

```python
import functools

import jax
import jax.numpy as jnp
import numpy as np
import jax.experimental.pallas as pl
import jax.experimental.pallas.tpu as pltpu

F32 = jnp.float32
BF16 = jnp.bfloat16
U32 = jnp.uint32

C = 128


def _dft_mats():
    f = np.arange(C, dtype=np.float64)[:, None] + 0.5
    t = np.arange(C, dtype=np.float64)[None, :]
    ang = 2.0 * np.pi * f * t / (2 * C)
    fwd = np.concatenate([np.cos(ang), -np.sin(ang)], axis=0)
    inv = np.concatenate([np.cos(ang).T, -np.sin(ang).T], axis=1) * (2.0 / (2 * C))
    return fwd.astype(np.float32), inv.astype(np.float32)


def _nt(a, b):
    return jax.lax.dot_general(a, b, (((1,), (1,)), ((), ())), preferred_element_type=F32)


def _nn(a, b):
    return jnp.dot(a, b, preferred_element_type=F32)


def _kernel(q_hbm, k_hbm, v_hbm, shift_ref, ssmk_hbm, ssmd_ref, mem0_ref,
            wq_hbm, wk_hbm, wv_hbm, wo_hbm, gate_ref, f_ref, fi_ref,
            out_hbm,
            qbuf, kbuf, vbuf, sbuf, raw, wqkv, wo, abuf, gbuf, obuf,
            dskip, kvbuf, asp, ksp, ysp, membuf, pend, pendo, o32, pacc,
            sem_in, sem_wo, sem_out,
            *, S, D, H, seg, M):
    NG = D // 128
    NCH = S // C
    DCH = D // NG
    HP = H // 2
    CR = DCH * HP

    def in_copies(g):
        sl = pl.ds(pl.multiple_of(g * 128, 128), 128)
        rows = pl.ds(pl.multiple_of(g * CR, CR), CR)
        cps = [pltpu.make_async_copy(k_hbm.at[:, sl], kbuf.at[g], sem_in.at[0, g]),
               pltpu.make_async_copy(v_hbm.at[:, sl], vbuf.at[g], sem_in.at[1, g]),
               pltpu.make_async_copy(ssmk_hbm.at[sl, :], sbuf.at[g], sem_in.at[2, g]),
               pltpu.make_async_copy(q_hbm.at[:, sl], qbuf.at[g], sem_in.at[3, g])]
        for i, w in enumerate((wq_hbm, wk_hbm, wv_hbm)):
            cps.append(pltpu.make_async_copy(
                w.bitcast(U32).at[rows, :], raw.at[i, g], sem_in.at[4 + i, g]))
        return cps

    def wo_copy(n):
        return pltpu.make_async_copy(wo_hbm.at[:, pl.ds(n * 128, 128)], wo.at[n], sem_wo.at[n])

    AHEAD = 2
    for g in range(AHEAD):
        for cp in in_copies(g):
            cp.start()

    ks = shift_ref.shape[0]
    dskip[...] = ssmd_ref[...].astype(F32).reshape(1, D)
    fmat = f_ref[...]
    sgn = 1.0 - 2.0 * (jax.lax.broadcasted_iota(jnp.int32, (8, 128), 0) % 2).astype(F32)

    def repack(g, i, b):
        x = raw[i, g, b * 16 * HP:(b + 1) * 16 * HP, :].reshape(8, 2, HP // 8, 8, 128)
        dst = pl.ds(pl.multiple_of(g * (DCH // 2) + b * 8, 8), 8)
        for t in range(HP // 8):
            ev = jnp.transpose(x[:, 0, t], (1, 0, 2))
            od = jnp.transpose(x[:, 1, t], (1, 0, 2))
            for j in range(8):
                h = i * H + 2 * (8 * t + j)
                wqkv[h, dst, :] = (ev[j] & 0xFFFF) | (od[j] << 16)
                wqkv[h + 1, dst, :] = (ev[j] >> 16) | (od[j] & U32(0xFFFF0000))

    def conv_group(g, _):
        for cp in in_copies(g):
            cp.wait()

        @pl.when(g + AHEAD < NG)
        def _():
            for cp in in_copies(g + AHEAD):
                cp.start()

        @pl.when(g + AHEAD == NG)
        def _():
            for n in range(NG):
                wo_copy(n).start()

        lanes = pl.ds(pl.multiple_of(g * 128, 128), 128)
        tp = shift_ref[:, lanes].astype(F32)
        dvec = dskip[:, lanes]
        for j in range(NCH):
            cur = kbuf[g, j * C:(j + 1) * C, :].astype(F32)
            if j == 0:
                prev = jnp.zeros((16, 128), F32)
            else:
                prev = kbuf[g, j * C - 16:j * C, :].astype(F32)
            ext = jnp.concatenate([prev, cur], axis=0)
            acc = cur * tp[0:1, :]
            for u in range(1, ks):
                acc = acc + ext[16 - u:16 - u + C, :] * tp[u:u + 1, :]
            kv = (acc * vbuf[g, j * C:(j + 1) * C, :].astype(F32)).astype(BF16)
            kvbuf[j * C:(j + 1) * C, :] = kv
            asp[j] = _nn(fmat, kv)
            ksp[j] = _nt(fmat, sbuf[g, :, j * C:(j + 1) * C])
            for bi in range(j * 3 * DCH // (16 * NCH), (j + 1) * 3 * DCH // (16 * NCH)):
                repack(g, bi // (DCH // 16), bi % (DCH // 16))

        def freq_block(fb, _):
            rr = pl.ds(pl.multiple_of(fb * 8, 8), 8)
            ri = pl.ds(pl.multiple_of(C + fb * 8, 8), 8)
            prev_z = None
            IB = 4
            for i0 in range(0, NCH, IB):
                kc = {}
                zr = [None] * IB
                zi = [None] * IB
                for j in range(i0 + IB):
                    ar, ai = asp[j, rr, :], asp[j, ri, :]
                    for ii in range(IB):
                        m = i0 + ii - j
                        if m < 0:
                            continue
                        if m not in kc:
                            kc[m] = (ksp[m, rr, :], ksp[m, ri, :])
                        kr, kim = kc[m]
                        pr = ar * kr - ai * kim
                        pi = ar * kim + ai * kr
                        zr[ii] = pr if zr[ii] is None else zr[ii] + pr
                        zi[ii] = pi if zi[ii] is None else zi[ii] + pi
                for ii in range(IB):
                    if prev_z is None:
                        yr, yi = zr[ii], zi[ii]
                    else:
                        yr = zr[ii] - sgn * prev_z[1]
                        yi = zi[ii] + sgn * prev_z[0]
                    prev_z = (zr[ii], zi[ii])
                    ysp[i0 + ii, rr, :] = yr
                    ysp[i0 + ii, ri, :] = yi
            return 0

        jax.lax.fori_loop(0, C // 8, freq_block, 0)

        fimat = fi_ref[...]
        for j in range(NCH):
            y = _nn(fimat, ysp[j].astype(BF16)).astype(BF16).astype(F32)
            kv = kvbuf[j * C:(j + 1) * C, :].astype(F32)
            y = (y + (kv * dvec).astype(BF16).astype(F32)).astype(BF16).astype(F32)
            qv = qbuf[g, j * C:(j + 1) * C, :].astype(F32)
            abuf[g, j * C:(j + 1) * C, :] = (qv * y).astype(BF16)
        return 0

    jax.lax.fori_loop(0, NG, conv_group, 0)

    gw = jnp.broadcast_to(gate_ref[...].reshape(1, D), (128, D))
    RB = 256

    def gate_blk(i, _):
        rows = pl.ds(pl.multiple_of(i * RB, RB), RB)
        x = jnp.concatenate([qbuf[g, rows, :] for g in range(NG)], axis=1)
        z = _nt(x, gw)
        gbuf[rows, :] = jax.nn.sigmoid(z)
        return 0

    jax.lax.fori_loop(0, S // RB, gate_blk, 0)

    for n in range(NG):
        wo_copy(n).wait()

    membuf[...] = mem0_ref[...].astype(F32)
    L = M + seg
    scale = 128 ** -0.5
    row = jax.lax.broadcasted_iota(jnp.int32, (L, 48), 0)
    col = jax.lax.broadcasted_iota(jnp.int32, (L, 48), 1)
    mask = (col < L) & ((row < M) | (row >= col))

    LAG = 3
    HS = 16
    E0 = 4

    def step(u, even):
        r0 = pl.multiple_of(u * 2 * seg, 2 * seg)
        if even:
            xs, nx = r0, 40
        else:
            xs, nx = r0 + 40, 24
        xs = pl.multiple_of(xs, 8)
        rows_m = M + nx
        lhs = jnp.concatenate(
            [jnp.concatenate([membuf[:, g * 128:(g + 1) * 128],
                              qbuf[g, pl.ds(xs, nx), :].astype(F32)], axis=0)
             for g in range(NG)], axis=1).astype(BF16)

        rows_o = 32 if even else 48
        nb = rows_o - M
        b0 = pl.multiple_of(r0 if even else r0 + 24, 8)
        brow = pl.ds(b0, nb)
        qkv, es = {}, {}

        def proj(h):
            res = []
            for i in range(3):
                r = _nn(lhs, pltpu.bitcast(wqkv[i * H + h], BF16))
                if even:
                    pend[i * H + h] = r[40:48]
                    full = r
                else:
                    full = jnp.concatenate(
                        [r[0:8], pend[i * H + h], r[8:32], jnp.zeros((8, 128), F32)], axis=0)
                res.append(full.astype(BF16))
            qkv[h] = res

        def scores(h):
            qh, kh, _ = qkv[h]
            s = _nt(qh, kh)[:L]
            s = jnp.where(mask, s, -1e9 / scale)
            mx = jnp.max(s, axis=1, keepdims=True)
            e = jnp.exp((s - mx) * scale)
            l = jnp.sum(e, axis=1, keepdims=True)
            e = jnp.concatenate([e, jnp.zeros((48 - L, 48), F32)], axis=0).astype(BF16)
            es[h] = (e, 1.0 / l)

        def attend(h):
            e, rl = es.pop(h)
            o = _nn(e, qkv.pop(h)[2])[:L] * rl
            if even:
                pendo[h] = o[32:40]
                o32[h, 0:16, :] = pltpu.bitcast(o[0:32].astype(BF16), U32)
            else:
                oo = jnp.concatenate([o[0:8], pendo[h], o[8:40]], axis=0)
                o32[h] = pltpu.bitcast(oo.astype(BF16), U32)

        def out_proj(n, h0, h1):
            ol = jnp.concatenate(
                [pltpu.bitcast(o32[h, 0:rows_o // 2, :], BF16) for h in range(h0, h1)], axis=1)
            return _nn(ol, wo[n, h0 * 128:h1 * 128, :])

        def early_out(ns):
            for n in ns:
                pacc[0:rows_o, n * 128:(n + 1) * 128] = out_proj(n, 0, HS)

        for t in range(H + 1 + LAG):
            if t < H:
                proj(t)
            if t == H:
                early_out(range(0, E0))
            if 0 <= t - 1 < H:
                scores(t - 1)
            if t == H:
                early_out(range(E0, NG))
            if 0 <= t - 1 - LAG < H:
                attend(t - 1 - LAG)

        gv = gbuf[brow, :]
        for n in range(NG):
            r = out_proj(n, HS, H) + pacc[0:rows_o, n * 128:(n + 1) * 128]
            r = r.astype(BF16).astype(F32)
            membuf[:, n * 128:(n + 1) * 128] = r[0:M]
            b = r[M:]
            a = abuf[n, brow, :].astype(F32)
            obuf[brow, n * 128:(n + 1) * 128] = (b + gv * (a - b)).astype(BF16)

    def double_step(u, _):
        step(u, True)
        step(u, False)
        rows = pl.ds(pl.multiple_of(u * 2 * seg, 2 * seg), 2 * seg)
        pltpu.make_async_copy(obuf.at[rows, :], out_hbm.at[rows, :], sem_out).start()
        return 0

    jax.lax.fori_loop(0, S // (2 * seg), double_step, 0)
    pltpu.make_async_copy(obuf, out_hbm, sem_out).wait()


@functools.partial(jax.jit, static_argnames=("B_seg_len",))
def pallas_gated_mix__ssm_conv_h3__memory_aug_recurrent_mem_tr__prompt_kernel(
    A_q: jax.Array,
    A_k: jax.Array,
    A_v: jax.Array,
    A_shift_k: jax.Array,
    A_ssm_k: jax.Array,
    A_ssm_D: jax.Array,
    B_x: jax.Array,
    B_mem0: jax.Array,
    B_Wq: jax.Array,
    B_Wk: jax.Array,
    B_Wv: jax.Array,
    B_Wo: jax.Array,
    B_seg_len,
    gate_w: jax.Array,
):
    del B_x
    Bn, S, D = A_q.shape
    Dm, H, Dh = B_Wq.shape
    M = B_mem0.shape[1]
    seg = int(B_seg_len)
    assert Bn == 1 and Dh == 128 and Dm == D and M == 8 and seg == 32
    assert S % (2 * seg) == 0 and S % 256 == 0 and D % 128 == 0 and D // 128 >= 2 and H % 16 == 0
    NG = D // 128
    fwd, inv = _dft_mats()

    any_spec = pl.BlockSpec(memory_space=pl.ANY)
    vmem_spec = pl.BlockSpec(memory_space=pltpu.VMEM)
    out = pl.pallas_call(
        functools.partial(_kernel, S=S, D=D, H=H, seg=seg, M=M),
        out_shape=jax.ShapeDtypeStruct((S, D), A_q.dtype),
        in_specs=[any_spec, any_spec, any_spec, vmem_spec, any_spec, vmem_spec, vmem_spec,
                  any_spec, any_spec, any_spec, any_spec, vmem_spec, vmem_spec, vmem_spec],
        out_specs=any_spec,
        scratch_shapes=[
            pltpu.VMEM((NG, S, 128), BF16),
            pltpu.VMEM((NG, S, 128), BF16),
            pltpu.VMEM((NG, S, 128), BF16),
            pltpu.VMEM((NG, 128, S), BF16),
            pltpu.VMEM((3, NG, D * H // (2 * NG), 128), U32),
            pltpu.VMEM((3 * H, D // 2, 128), U32),
            pltpu.VMEM((NG, H * Dh, 128), BF16),
            pltpu.VMEM((NG, S, 128), BF16),
            pltpu.VMEM((S, 128), F32),
            pltpu.VMEM((S, D), BF16),
            pltpu.VMEM((1, D), F32),
            pltpu.VMEM((S, 128), BF16),
            pltpu.VMEM((S // C, 2 * C, 128), F32),
            pltpu.VMEM((S // C, 2 * C, 128), F32),
            pltpu.VMEM((S // C, 2 * C, 128), F32),
            pltpu.VMEM((M, D), F32),
            pltpu.VMEM((3 * H, 8, 128), F32),
            pltpu.VMEM((H, 8, 128), F32),
            pltpu.VMEM((H, 24, 128), U32),
            pltpu.VMEM((48, D), F32),
            pltpu.SemaphoreType.DMA((7, NG)),
            pltpu.SemaphoreType.DMA((NG,)),
            pltpu.SemaphoreType.DMA(()),
        ],
        compiler_params=pltpu.CompilerParams(vmem_limit_bytes=120 * 1024 * 1024),
    )(
        A_q.reshape(S, D), A_k.reshape(S, D), A_v.reshape(S, D), A_shift_k.T, A_ssm_k,
        A_ssm_D, B_mem0.reshape(M, D),
        B_Wq.reshape(D * H, Dh), B_Wk.reshape(D * H, Dh), B_Wv.reshape(D * H, Dh),
        B_Wo.reshape(H * Dh, D), gate_w,
        jnp.asarray(fwd, BF16), jnp.asarray(inv, BF16),
    )
    return out.reshape(Bn, S, D)
```

```python
import functools

import jax
import jax.numpy as jnp
import numpy as np
import jax.experimental.pallas as pl
import jax.experimental.pallas.tpu as pltpu

F32 = jnp.float32
BF16 = jnp.bfloat16
U32 = jnp.uint32

NSLOT = 3
C = 128


def _dft_mats():
    f = np.arange(C, dtype=np.float64)[:, None] + 0.5
    t = np.arange(C, dtype=np.float64)[None, :]
    ang = 2.0 * np.pi * f * t / (2 * C)
    fwd = np.concatenate([np.cos(ang), -np.sin(ang)], axis=0)
    inv = np.concatenate([np.cos(ang).T, -np.sin(ang).T], axis=1) * (2.0 / (2 * C))
    return fwd.astype(np.float32), inv.astype(np.float32)


def _nt(a, b):
    return jax.lax.dot_general(a, b, (((1,), (1,)), ((), ())), preferred_element_type=F32)


def _nn(a, b):
    return jnp.dot(a, b, preferred_element_type=F32)


def _push(stack, x):
    n = 1
    while stack and stack[-1][0] == n:
        m, y = stack.pop()
        x, n = y + x, n + m
    stack.append((n, x))


def _total(stack):
    x = stack[-1][1]
    for _, y in reversed(stack[:-1]):
        x = y + x
    return x


def _kernel(q_hbm, k_hbm, v_hbm, shift_ref, ssmk_hbm, ssmd_ref, mem0_ref,
            wq_hbm, wk_hbm, wv_hbm, wo_hbm, gate_ref, f_ref, fi_ref,
            out_hbm,
            qbuf, kbuf, vbuf, sbuf, raw, wqkv, wo, abuf, gbuf, obuf,
            dskip, pre, xpre, kvbuf, asp, ksp, ysp, membuf, pendo, o32, pacc,
            sem_in, sem_wo, sem_out,
            *, S, D, H, seg, M):
    NG = D // 128
    NCH = S // C
    DCH = D // NG
    HP = H // 2
    CR = DCH * HP
    NSEG = S // seg
    PRE = NSEG * 8

    def in_copies(g):
        g = jnp.int32(g)
        sl = pl.ds(pl.multiple_of(g * 128, 128), 128)
        rows = pl.ds(pl.multiple_of(g * CR, CR), CR)
        cps = [pltpu.make_async_copy(k_hbm.at[:, sl], kbuf.at[g], sem_in.at[0, g]),
               pltpu.make_async_copy(v_hbm.at[:, sl], vbuf.at[g], sem_in.at[1, g]),
               pltpu.make_async_copy(ssmk_hbm.at[sl, :], sbuf.at[g], sem_in.at[2, g]),
               pltpu.make_async_copy(q_hbm.at[:, sl], qbuf.at[g], sem_in.at[3, g])]
        for i, w in enumerate((wq_hbm, wk_hbm, wv_hbm)):
            cps.append(pltpu.make_async_copy(
                w.bitcast(U32).at[rows, :], raw.at[i, jax.lax.rem(g, NSLOT)], sem_in.at[4 + i, g]))
        return cps

    def wo_copy(n):
        return pltpu.make_async_copy(wo_hbm.at[:, pl.ds(n * 128, 128)], wo.at[n], sem_wo.at[n])

    AHEAD = NSLOT - 1
    for g in range(AHEAD):
        for cp in in_copies(g):
            cp.start()

    def zero_pre(i, _):
        pre[i] = jnp.zeros((PRE, 128), F32)
        return 0

    jax.lax.fori_loop(0, 3 * H, zero_pre, 0)

    ks = shift_ref.shape[0]
    dskip[...] = ssmd_ref[...].astype(F32).reshape(1, D)
    fmat = f_ref[...]
    sgn = 1.0 - 2.0 * (jax.lax.broadcasted_iota(jnp.int32, (8, 128), 0) % 2).astype(F32)

    def repack(g, i, b):
        src = pl.ds(pl.multiple_of(b * 16 * HP, 16 * HP), 16 * HP)
        x = raw[i, jax.lax.rem(g, NSLOT), src, :].reshape(8, 2, HP // 8, 8, 128)
        dst = pl.ds(pl.multiple_of(g * (DCH // 2) + b * 8, 8), 8)
        for t in range(HP // 8):
            ev = jnp.transpose(x[:, 0, t], (1, 0, 2))
            od = jnp.transpose(x[:, 1, t], (1, 0, 2))
            for j in range(8):
                h = i * H + 2 * (8 * t + j)
                wqkv[h, dst, :] = (ev[j] & 0xFFFF) | (od[j] << 16)
                wqkv[h + 1, dst, :] = (ev[j] >> 16) | (od[j] & U32(0xFFFF0000))

    NSB = 8

    def gather_pre(g):
        for sgi in range(0, NSEG, 2):
            xpre[sgi * 4:(sgi + 2) * 4, :] = pltpu.bitcast(jnp.concatenate(
                [qbuf[g, sgi * seg:sgi * seg + 8, :],
                 qbuf[g, (sgi + 1) * seg:(sgi + 1) * seg + 8, :]], axis=0), U32)

    E_ORDER = 2

    def pre_tiles(g, sb, tts):
        krows = pl.ds(pl.multiple_of(g * 64, 64), 64)
        for tt in tts:
            idx = sb * (3 * H // NSB) + tt
            pre[idx] = pre[idx] + _nn(pltpu.bitcast(xpre[...], BF16),
                                        pltpu.bitcast(wqkv[idx, krows, :], BF16))

    def conv_group(g, _, with_pre=True):
        for cp in in_copies(g):
            cp.wait()

        @pl.when(g + AHEAD < NG)
        def _():
            for cp in in_copies(g + AHEAD):
                cp.start()

        @pl.when(g + AHEAD == NG)
        def _():
            for n in range(NG):
                wo_copy(n).start()

        lanes = pl.ds(pl.multiple_of(g * 128, 128), 128)
        tp = shift_ref[:, lanes].astype(F32)
        dvec = dskip[:, lanes]
        for j in range(NCH):
            cur = kbuf[g, j * C:(j + 1) * C, :].astype(F32)
            if j == 0:
                prev = jnp.zeros((16, 128), F32)
            else:
                prev = kbuf[g, j * C - 16:j * C, :].astype(F32)
            ext = jnp.concatenate([prev, cur], axis=0)
            acc = cur * tp[0:1, :]
            for u in range(1, ks):
                acc = acc + ext[16 - u:16 - u + C, :] * tp[u:u + 1, :]
            kv = (acc * vbuf[g, j * C:(j + 1) * C, :].astype(F32)).astype(BF16)
            kvbuf[j * C:(j + 1) * C, :] = kv
            sa = _nn(fmat, kv)
            asp[j, 0:2 * C, :] = sa
            asp[j, 2 * C:3 * C, :] = sa[0:C] + sa[C:2 * C]
            sk = _nt(fmat, sbuf[g, :, j * C:(j + 1) * C])
            ksp[j, 0:C, :] = sk[0:C]
            ksp[j, C:2 * C, :] = sk[C:2 * C] - sk[0:C]
            ksp[j, 2 * C:3 * C, :] = sk[C:2 * C] + sk[0:C]

        if with_pre:
            gather_pre(g - 1)

        def super_block(sb, _):
            nf = C // 8 // NSB
            nt = 3 * H // NSB
            order = E_ORDER
            if order == 0:
                if with_pre:
                    pre_tiles(g - 1, sb, range(nt))
                for b in range(DCH // 16 // NSB):
                    for i in range(3):
                        repack(g, i, sb * (DCH // 16 // NSB) + b)
                for fi in range(nf):
                    freq_block(sb * nf + fi)
            elif order == 1:
                for fi in range(nf):
                    freq_block(sb * nf + fi)
                for b in range(DCH // 16 // NSB):
                    for i in range(3):
                        repack(g, i, sb * (DCH // 16 // NSB) + b)
                if with_pre:
                    pre_tiles(g - 1, sb, range(nt))
            else:
                for fi in range(nf):
                    if with_pre:
                        pre_tiles(g - 1, sb, range(fi * nt // nf, (fi + 1) * nt // nf))
                    freq_block(sb * nf + fi)
                for b in range(DCH // 16 // NSB):
                    for i in range(3):
                        repack(g, i, sb * (DCH // 16 // NSB) + b)
            return 0

        def freq_block(fb):
            rr = pl.ds(pl.multiple_of(fb * 8, 8), 8)
            ri = pl.ds(pl.multiple_of(C + fb * 8, 8), 8)
            rs = pl.ds(pl.multiple_of(2 * C + fb * 8, 8), 8)
            prev_z = None
            IB = 4
            for i0 in range(0, NCH, IB):
                kc = {}
                acc = [[[], [], []] for _ in range(IB)]
                for j in range(i0 + IB):
                    ar, ai, asum = asp[j, rr, :], asp[j, ri, :], asp[j, rs, :]
                    for ii in range(IB):
                        m = i0 + ii - j
                        if m < 0:
                            continue
                        if m not in kc:
                            kc[m] = (ksp[m, rr, :], ksp[m, ri, :], ksp[m, rs, :])
                        kr, kdif, ksum = kc[m]
                        _push(acc[ii][0], kr * asum)
                        _push(acc[ii][1], ar * kdif)
                        _push(acc[ii][2], ai * ksum)
                acc = [[_total(x) for x in z] for z in acc]
                zr = [z[0] - z[2] for z in acc]
                zi = [z[0] + z[1] for z in acc]
                for ii in range(IB):
                    if prev_z is None:
                        yr, yi = zr[ii], zi[ii]
                    else:
                        yr = zr[ii] - sgn * prev_z[1]
                        yi = zi[ii] + sgn * prev_z[0]
                    prev_z = (zr[ii], zi[ii])
                    ysp[i0 + ii, rr, :] = yr
                    ysp[i0 + ii, ri, :] = yi

        jax.lax.fori_loop(0, NSB, super_block, 0)

        fimat = fi_ref[...]
        for j in range(NCH):
            y = _nn(fimat, ysp[j].astype(BF16)).astype(BF16).astype(F32)
            kv = kvbuf[j * C:(j + 1) * C, :].astype(F32)
            y = (y + (kv * dvec).astype(BF16).astype(F32)).astype(BF16).astype(F32)
            qv = qbuf[g, j * C:(j + 1) * C, :].astype(F32)
            abuf[g, j * C:(j + 1) * C, :] = (qv * y).astype(BF16)
        return 0

    conv_group(jnp.int32(0), 0, with_pre=False)
    jax.lax.fori_loop(1, NG, conv_group, 0)
    gather_pre(NG - 1)

    def last_pre(sb, _):
        pre_tiles(jnp.int32(NG - 1), sb, range(3 * H // NSB))
        return 0

    jax.lax.fori_loop(0, NSB, last_pre, 0)

    gw = jnp.broadcast_to(gate_ref[...].reshape(1, D), (128, D))
    RB = 256

    def gate_blk(i, _):
        rows = pl.ds(pl.multiple_of(i * RB, RB), RB)
        x = jnp.concatenate([qbuf[g, rows, :] for g in range(NG)], axis=1)
        z = _nt(x, gw)
        gbuf[rows, :] = jax.nn.sigmoid(z)
        return 0

    jax.lax.fori_loop(0, S // RB, gate_blk, 0)

    for n in range(NG):
        wo_copy(n).wait()

    membuf[...] = mem0_ref[...].astype(F32)
    L = M + seg
    scale = 128 ** -0.5
    row = jax.lax.broadcasted_iota(jnp.int32, (L, 48), 0)
    col = jax.lax.broadcasted_iota(jnp.int32, (L, 48), 1)
    mask = (col < L) & ((row < M) | (row >= col))

    LAG = 4
    HS = 16
    E0 = 4

    def step(u, even):
        r0 = pl.multiple_of(u * 2 * seg, 2 * seg)
        xs, nx = pl.multiple_of(r0 + (8 if even else seg + 8), 8), seg - 8
        prow = pl.ds(pl.multiple_of(u * 16 + (0 if even else 8), 8), 8)
        lhs = jnp.concatenate(
            [jnp.concatenate([membuf[:, g * 128:(g + 1) * 128],
                              qbuf[g, pl.ds(xs, nx), :].astype(F32)], axis=0)
             for g in range(NG)], axis=1).astype(BF16)

        rows_o = 32 if even else 48
        nb = rows_o - M
        b0 = pl.multiple_of(r0 if even else r0 + 24, 8)
        brow = pl.ds(b0, nb)
        qkv, es = {}, {}

        def proj(h):
            res = []
            for i in range(3):
                r = _nn(lhs, pltpu.bitcast(wqkv[i * H + h], BF16))
                full = jnp.concatenate(
                    [r[0:M], pre[i * H + h, prow, :], r[M:], jnp.zeros((8, 128), F32)], axis=0)
                res.append(full.astype(BF16))
            qkv[h] = res

        def scores(h):
            qh, kh, _ = qkv[h]
            s = _nt(qh, kh)[:L]
            s = jnp.where(mask, s, -1e9 / scale)
            mx = jnp.max(s, axis=1, keepdims=True)
            e = jnp.exp((s - mx) * scale)
            l = jnp.sum(e, axis=1, keepdims=True)
            e = jnp.concatenate([e, jnp.zeros((48 - L, 48), F32)], axis=0).astype(BF16)
            es[h] = (e, 1.0 / l)

        def attend(h):
            e, rl = es.pop(h)
            o = _nn(e, qkv.pop(h)[2])[:L] * rl
            if even:
                pendo[h] = o[32:40]
                o32[h, 0:16, :] = pltpu.bitcast(o[0:32].astype(BF16), U32)
            else:
                oo = jnp.concatenate([o[0:8], pendo[h], o[8:40]], axis=0)
                o32[h] = pltpu.bitcast(oo.astype(BF16), U32)

        def out_proj(n, h0, h1):
            ol = jnp.concatenate(
                [pltpu.bitcast(o32[h, 0:rows_o // 2, :], BF16) for h in range(h0, h1)], axis=1)
            return _nn(ol, wo[n, h0 * 128:h1 * 128, :])

        def early_out(ns):
            for n in ns:
                pacc[0:rows_o, n * 128:(n + 1) * 128] = out_proj(n, 0, HS)

        for t in range(H + 1 + LAG):
            if t < H:
                proj(t)
            if t == H:
                early_out(range(0, E0))
            if 0 <= t - 1 < H:
                scores(t - 1)
            if t == H:
                early_out(range(E0, NG))
            if 0 <= t - 1 - LAG < H:
                attend(t - 1 - LAG)

        gv = gbuf[brow, :]
        for n in range(NG):
            r = out_proj(n, HS, H) + pacc[0:rows_o, n * 128:(n + 1) * 128]
            r = r.astype(BF16).astype(F32)
            membuf[:, n * 128:(n + 1) * 128] = r[0:M]
            b = r[M:]
            a = abuf[n, brow, :].astype(F32)
            obuf[brow, n * 128:(n + 1) * 128] = (b + gv * (a - b)).astype(BF16)

    def double_step(u, _):
        step(u, True)
        step(u, False)
        rows = pl.ds(pl.multiple_of(u * 2 * seg, 2 * seg), 2 * seg)
        pltpu.make_async_copy(obuf.at[rows, :], out_hbm.at[rows, :], sem_out).start()
        return 0

    jax.lax.fori_loop(0, S // (2 * seg), double_step, 0)
    pltpu.make_async_copy(obuf, out_hbm, sem_out).wait()


@functools.partial(jax.jit, static_argnames=("B_seg_len",))
def pallas_gated_mix__ssm_conv_h3__memory_aug_recurrent_mem_tr__prompt_kernel(
    A_q: jax.Array,
    A_k: jax.Array,
    A_v: jax.Array,
    A_shift_k: jax.Array,
    A_ssm_k: jax.Array,
    A_ssm_D: jax.Array,
    B_x: jax.Array,
    B_mem0: jax.Array,
    B_Wq: jax.Array,
    B_Wk: jax.Array,
    B_Wv: jax.Array,
    B_Wo: jax.Array,
    B_seg_len,
    gate_w: jax.Array,
):
    del B_x
    Bn, S, D = A_q.shape
    Dm, H, Dh = B_Wq.shape
    M = B_mem0.shape[1]
    seg = int(B_seg_len)
    assert Bn == 1 and Dh == 128 and Dm == D and M == 8 and seg == 32
    assert S % (2 * seg) == 0 and S % 256 == 0 and D % 128 == 0 and D // 128 >= 2 and H % 16 == 0
    NG = D // 128
    fwd, inv = _dft_mats()

    any_spec = pl.BlockSpec(memory_space=pl.ANY)
    vmem_spec = pl.BlockSpec(memory_space=pltpu.VMEM)
    out = pl.pallas_call(
        functools.partial(_kernel, S=S, D=D, H=H, seg=seg, M=M),
        out_shape=jax.ShapeDtypeStruct((S, D), A_q.dtype),
        in_specs=[any_spec, any_spec, any_spec, vmem_spec, any_spec, vmem_spec, vmem_spec,
                  any_spec, any_spec, any_spec, any_spec, vmem_spec, vmem_spec, vmem_spec],
        out_specs=any_spec,
        scratch_shapes=[
            pltpu.VMEM((NG, S, 128), BF16),
            pltpu.VMEM((NG, S, 128), BF16),
            pltpu.VMEM((NG, S, 128), BF16),
            pltpu.VMEM((NG, 128, S), BF16),
            pltpu.VMEM((3, NSLOT, D * H // (2 * NG), 128), U32),
            pltpu.VMEM((3 * H, D // 2, 128), U32),
            pltpu.VMEM((NG, H * Dh, 128), BF16),
            pltpu.VMEM((NG, S, 128), BF16),
            pltpu.VMEM((S, 128), F32),
            pltpu.VMEM((S, D), BF16),
            pltpu.VMEM((1, D), F32),
            pltpu.VMEM((3 * H, S // seg * 8, 128), F32),
            pltpu.VMEM((S // seg * 4, 128), U32),
            pltpu.VMEM((S, 128), BF16),
            pltpu.VMEM((S // C, 3 * C, 128), F32),
            pltpu.VMEM((S // C, 3 * C, 128), F32),
            pltpu.VMEM((S // C, 2 * C, 128), F32),
            pltpu.VMEM((M, D), F32),
            pltpu.VMEM((H, 8, 128), F32),
            pltpu.VMEM((H, 24, 128), U32),
            pltpu.VMEM((48, D), F32),
            pltpu.SemaphoreType.DMA((7, NG)),
            pltpu.SemaphoreType.DMA((NG,)),
            pltpu.SemaphoreType.DMA(()),
        ],
        compiler_params=pltpu.CompilerParams(vmem_limit_bytes=120 * 1024 * 1024),
    )(
        A_q.reshape(S, D), A_k.reshape(S, D), A_v.reshape(S, D), A_shift_k.T, A_ssm_k,
        A_ssm_D, B_mem0.reshape(M, D),
        B_Wq.reshape(D * H, Dh), B_Wk.reshape(D * H, Dh), B_Wv.reshape(D * H, Dh),
        B_Wo.reshape(H * Dh, D), gate_w,
        jnp.asarray(fwd, BF16), jnp.asarray(inv, BF16),
    )
    return out.reshape(Bn, S, D)
```

```python
import functools

import jax
import jax.numpy as jnp
import numpy as np
import jax.experimental.pallas as pl
import jax.experimental.pallas.tpu as pltpu

F32 = jnp.float32
BF16 = jnp.bfloat16
U32 = jnp.uint32

NSLOT = 3
C = 128


def _dft_mats():
    f = np.arange(C, dtype=np.float64)[:, None] + 0.5
    t = np.arange(C, dtype=np.float64)[None, :]
    ang = 2.0 * np.pi * f * t / (2 * C)
    fwd = np.concatenate([np.cos(ang), -np.sin(ang)], axis=0)
    inv = np.concatenate([np.cos(ang).T, -np.sin(ang).T], axis=1) * (2.0 / (2 * C))
    return fwd.astype(np.float32), inv.astype(np.float32)


def _nt(a, b):
    return jax.lax.dot_general(a, b, (((1,), (1,)), ((), ())), preferred_element_type=F32)


def _nn(a, b):
    return jnp.dot(a, b, preferred_element_type=F32)


def _push(stack, x):
    n = 1
    while stack and stack[-1][0] == n:
        m, y = stack.pop()
        x, n = y + x, n + m
    stack.append((n, x))


def _total(stack):
    x = stack[-1][1]
    for _, y in reversed(stack[:-1]):
        x = y + x
    return x


def _kernel(q_hbm, k_hbm, v_hbm, shift_ref, ssmk_hbm, ssmd_ref, mem0_ref,
            wq_hbm, wk_hbm, wv_hbm, wo_hbm, gate_ref, f_ref, fi_ref,
            out_hbm,
            qbuf, kbuf, vbuf, sbuf, raw, wqkv, wo, abuf, gbuf, obuf,
            dskip, pre, xpre, kvbuf, asp, ksp, ysp, membuf, pendo, o32, pacc,
            sem_in, sem_wo, sem_out,
            *, S, D, H, seg, M):
    NG = D // 128
    NCH = S // C
    DCH = D // NG
    HP = H // 2
    CR = DCH * HP
    NSEG = S // seg
    PRE = NSEG * 8

    def in_copies(g):
        g = jnp.int32(g)
        sl = pl.ds(pl.multiple_of(g * 128, 128), 128)
        rows = pl.ds(pl.multiple_of(g * CR, CR), CR)
        cps = [pltpu.make_async_copy(k_hbm.at[:, sl], kbuf.at[g], sem_in.at[0, g]),
               pltpu.make_async_copy(v_hbm.at[:, sl], vbuf.at[g], sem_in.at[1, g]),
               pltpu.make_async_copy(ssmk_hbm.at[sl, :], sbuf.at[g], sem_in.at[2, g]),
               pltpu.make_async_copy(q_hbm.at[:, sl], qbuf.at[g], sem_in.at[3, g])]
        for i, w in enumerate((wq_hbm, wk_hbm, wv_hbm)):
            cps.append(pltpu.make_async_copy(
                w.bitcast(U32).at[rows, :], raw.at[i, jax.lax.rem(g, NSLOT)], sem_in.at[4 + i, g]))
        return cps

    def wo_copy(n):
        return pltpu.make_async_copy(
            wo_hbm.bitcast(U32).at[:, pl.ds(n * 128, 128)], wo.at[n], sem_wo.at[n])

    AHEAD = NSLOT - 1
    for g in range(AHEAD):
        for cp in in_copies(g):
            cp.start()

    def zero_pre(i, _):
        pre[i] = jnp.zeros((PRE, 128), F32)
        return 0

    jax.lax.fori_loop(0, 3 * H, zero_pre, 0)

    ks = shift_ref.shape[0]
    dskip[...] = ssmd_ref[...].astype(F32).reshape(1, D)
    fmat = f_ref[...]
    sgn = 1.0 - 2.0 * (jax.lax.broadcasted_iota(jnp.int32, (8, 128), 0) % 2).astype(F32)

    def repack(g, i, b):
        src = pl.ds(pl.multiple_of(b * 16 * HP, 16 * HP), 16 * HP)
        x = raw[i, jax.lax.rem(g, NSLOT), src, :].reshape(8, 2, HP // 8, 8, 128)
        dst = pl.ds(pl.multiple_of(g * (DCH // 2) + b * 8, 8), 8)
        for t in range(HP // 8):
            ev = jnp.transpose(x[:, 0, t], (1, 0, 2))
            od = jnp.transpose(x[:, 1, t], (1, 0, 2))
            for j in range(8):
                h = i * H + 2 * (8 * t + j)
                wqkv[h, dst, :] = (ev[j] & 0xFFFF) | (od[j] << 16)
                wqkv[h + 1, dst, :] = (ev[j] >> 16) | (od[j] & U32(0xFFFF0000))

    NSB = 8
    assert (DCH // 16) % NSB == 0 and (C // 8) % NSB == 0 and (3 * H) % NSB == 0

    def gather_pre(g):
        for sgi in range(0, NSEG, 2):
            xpre[sgi * 4:(sgi + 2) * 4, :] = pltpu.bitcast(jnp.concatenate(
                [qbuf[g, sgi * seg:sgi * seg + 8, :],
                 qbuf[g, (sgi + 1) * seg:(sgi + 1) * seg + 8, :]], axis=0), U32)

    def pre_tiles(g, sb, tts):
        krows = pl.ds(pl.multiple_of(g * 64, 64), 64)
        for tt in tts:
            idx = sb * (3 * H // NSB) + tt
            pre[idx] = pre[idx] + _nn(pltpu.bitcast(xpre[...], BF16),
                                        pltpu.bitcast(wqkv[idx, krows, :], BF16))

    def conv_group(g, _, with_pre=True):
        for cp in in_copies(g):
            cp.wait()

        @pl.when(g + AHEAD < NG)
        def _():
            for cp in in_copies(g + AHEAD):
                cp.start()

        @pl.when(g + AHEAD == NG)
        def _():
            for n in range(NG):
                wo_copy(n).start()

        lanes = pl.ds(pl.multiple_of(g * 128, 128), 128)
        tp = shift_ref[:, lanes].astype(F32)
        dvec = dskip[:, lanes]
        for j in range(NCH):
            cur = kbuf[g, j * C:(j + 1) * C, :].astype(F32)
            if j == 0:
                prev = jnp.zeros((16, 128), F32)
            else:
                prev = kbuf[g, j * C - 16:j * C, :].astype(F32)
            ext = jnp.concatenate([prev, cur], axis=0)
            acc = cur * tp[0:1, :]
            for u in range(1, ks):
                acc = acc + ext[16 - u:16 - u + C, :] * tp[u:u + 1, :]
            kv = (acc * vbuf[g, j * C:(j + 1) * C, :].astype(F32)).astype(BF16)
            kvbuf[j * C:(j + 1) * C, :] = kv
            sa = _nn(fmat, kv)
            asp[j, 0:2 * C, :] = sa
            asp[j, 2 * C:3 * C, :] = sa[0:C] + sa[C:2 * C]
            sk = _nt(fmat, sbuf[g, :, j * C:(j + 1) * C])
            ksp[j, 0:C, :] = sk[0:C]
            ksp[j, C:2 * C, :] = sk[C:2 * C] - sk[0:C]
            ksp[j, 2 * C:3 * C, :] = sk[C:2 * C] + sk[0:C]

        if with_pre:
            gather_pre(g - 1)

        def super_block(sb, _):
            nf = C // 8 // NSB
            nt = 3 * H // NSB
            for fi in range(nf):
                if with_pre:
                    pre_tiles(g - 1, sb, range(fi * nt // nf, (fi + 1) * nt // nf))
                freq_block(sb * nf + fi)
            for b in range(DCH // 16 // NSB):
                for i in range(3):
                    repack(g, i, sb * (DCH // 16 // NSB) + b)
            return 0

        def freq_block(fb):
            rr = pl.ds(pl.multiple_of(fb * 8, 8), 8)
            ri = pl.ds(pl.multiple_of(C + fb * 8, 8), 8)
            rs = pl.ds(pl.multiple_of(2 * C + fb * 8, 8), 8)
            prev_z = None
            IB = 4
            for i0 in range(0, NCH, IB):
                kc = {}
                acc = [[[], [], []] for _ in range(IB)]
                for j in range(i0 + IB):
                    ar, ai, asum = asp[j, rr, :], asp[j, ri, :], asp[j, rs, :]
                    for ii in range(IB):
                        m = i0 + ii - j
                        if m < 0:
                            continue
                        if m not in kc:
                            kc[m] = (ksp[m, rr, :], ksp[m, ri, :], ksp[m, rs, :])
                        kr, kdif, ksum = kc[m]
                        _push(acc[ii][0], kr * asum)
                        _push(acc[ii][1], ar * kdif)
                        _push(acc[ii][2], ai * ksum)
                acc = [[_total(x) for x in z] for z in acc]
                zr = [z[0] - z[2] for z in acc]
                zi = [z[0] + z[1] for z in acc]
                for ii in range(IB):
                    if prev_z is None:
                        yr, yi = zr[ii], zi[ii]
                    else:
                        yr = zr[ii] - sgn * prev_z[1]
                        yi = zi[ii] + sgn * prev_z[0]
                    prev_z = (zr[ii], zi[ii])
                    ysp[i0 + ii, rr, :] = yr
                    ysp[i0 + ii, ri, :] = yi

        jax.lax.fori_loop(0, NSB, super_block, 0)

        fimat = fi_ref[...]
        for j in range(NCH):
            y = _nn(fimat, ysp[j].astype(BF16)).astype(BF16).astype(F32)
            kv = kvbuf[j * C:(j + 1) * C, :].astype(F32)
            y = (y + (kv * dvec).astype(BF16).astype(F32)).astype(BF16).astype(F32)
            qv = qbuf[g, j * C:(j + 1) * C, :].astype(F32)
            abuf[g, j * C:(j + 1) * C, :] = (qv * y).astype(BF16)
        return 0

    conv_group(jnp.int32(0), 0, with_pre=False)
    jax.lax.fori_loop(1, NG, conv_group, 0)
    gather_pre(NG - 1)

    def last_pre(sb, _):
        pre_tiles(jnp.int32(NG - 1), sb, range(3 * H // NSB))
        return 0

    jax.lax.fori_loop(0, NSB, last_pre, 0)

    gw = jnp.broadcast_to(gate_ref[...].reshape(1, D), (128, D))
    RB = 256

    def gate_blk(i, _):
        rows = pl.ds(pl.multiple_of(i * RB, RB), RB)
        x = jnp.concatenate([qbuf[g, rows, :] for g in range(NG)], axis=1)
        z = _nt(x, gw)
        gbuf[rows, :] = jax.nn.sigmoid(z)
        return 0

    jax.lax.fori_loop(0, S // RB, gate_blk, 0)

    for n in range(NG):
        wo_copy(n).wait()

    membuf[...] = mem0_ref[...].astype(F32)
    L = M + seg
    scale = 128 ** -0.5
    row = jax.lax.broadcasted_iota(jnp.int32, (L, 48), 0)
    col = jax.lax.broadcasted_iota(jnp.int32, (L, 48), 1)
    mask = (col < L) & ((row < M) | (row >= col))

    LAG = 4
    HS = 16
    E0 = 4

    def step(u, even):
        r0 = pl.multiple_of(u * 2 * seg, 2 * seg)
        xs, nx = pl.multiple_of(r0 + (8 if even else seg + 8), 8), seg - 8
        prow = pl.ds(pl.multiple_of(u * 16 + (0 if even else 8), 8), 8)
        lhs = jnp.concatenate(
            [jnp.concatenate([membuf[:, g * 128:(g + 1) * 128],
                              qbuf[g, pl.ds(xs, nx), :].astype(F32)], axis=0)
             for g in range(NG)], axis=1).astype(BF16)

        rows_o = 32 if even else 48
        nb = rows_o - M
        b0 = pl.multiple_of(r0 if even else r0 + 24, 8)
        brow = pl.ds(b0, nb)
        qkv, es = {}, {}

        def proj(h):
            res = []
            for i in range(3):
                r = _nn(lhs, pltpu.bitcast(wqkv[i * H + h], BF16))
                full = jnp.concatenate(
                    [r[0:M], pre[i * H + h, prow, :], r[M:], jnp.zeros((8, 128), F32)], axis=0)
                res.append(full.astype(BF16))
            qkv[h] = res

        def scores(h):
            qh, kh, _ = qkv[h]
            s = _nt(qh, kh)[:L]
            s = jnp.where(mask, s, -1e9 / scale)
            mx = jnp.max(s, axis=1, keepdims=True)
            e = jnp.exp((s - mx) * scale)
            l = jnp.sum(e, axis=1, keepdims=True)
            e = jnp.concatenate([e, jnp.zeros((48 - L, 48), F32)], axis=0).astype(BF16)
            es[h] = (e, 1.0 / l)

        def attend(h):
            e, rl = es.pop(h)
            o = _nn(e, qkv.pop(h)[2])[:L] * rl
            if even:
                pendo[h] = o[32:40]
                o32[h, 0:16, :] = pltpu.bitcast(o[0:32].astype(BF16), U32)
            else:
                oo = jnp.concatenate([o[0:8], pendo[h], o[8:40]], axis=0)
                o32[h] = pltpu.bitcast(oo.astype(BF16), U32)

        def out_proj(n, h0, h1):
            ol = jnp.concatenate(
                [pltpu.bitcast(o32[h, 0:rows_o // 2, :], BF16) for h in range(h0, h1)], axis=1)
            return _nn(ol, pltpu.bitcast(wo[n, h0 * 64:h1 * 64, :], BF16))

        def early_out(ns):
            for n in ns:
                pacc[0:rows_o, n * 128:(n + 1) * 128] = out_proj(n, 0, HS)

        for t in range(H + 1 + LAG):
            if t < H:
                proj(t)
            if t == H:
                early_out(range(0, E0))
            if 0 <= t - 1 < H:
                scores(t - 1)
            if t == H:
                early_out(range(E0, NG))
            if 0 <= t - 1 - LAG < H:
                attend(t - 1 - LAG)

        gv = gbuf[brow, :]
        for n in range(NG):
            r = out_proj(n, HS, H) + pacc[0:rows_o, n * 128:(n + 1) * 128]
            r = r.astype(BF16).astype(F32)
            membuf[:, n * 128:(n + 1) * 128] = r[0:M]
            b = r[M:]
            a = abuf[n, brow, :].astype(F32)
            obuf[brow, n * 128:(n + 1) * 128] = (b + gv * (a - b)).astype(BF16)

    def double_step(u, _):
        step(u, True)
        step(u, False)
        rows = pl.ds(pl.multiple_of(u * 2 * seg, 2 * seg), 2 * seg)
        pltpu.make_async_copy(obuf.at[rows, :], out_hbm.at[rows, :], sem_out).start()
        return 0

    jax.lax.fori_loop(0, S // (2 * seg), double_step, 0)
    pltpu.make_async_copy(obuf, out_hbm, sem_out).wait()


@functools.partial(jax.jit, static_argnames=("B_seg_len",))
def pallas_gated_mix__ssm_conv_h3__memory_aug_recurrent_mem_tr__prompt_kernel(
    A_q: jax.Array,
    A_k: jax.Array,
    A_v: jax.Array,
    A_shift_k: jax.Array,
    A_ssm_k: jax.Array,
    A_ssm_D: jax.Array,
    B_x: jax.Array,
    B_mem0: jax.Array,
    B_Wq: jax.Array,
    B_Wk: jax.Array,
    B_Wv: jax.Array,
    B_Wo: jax.Array,
    B_seg_len,
    gate_w: jax.Array,
):
    del B_x
    Bn, S, D = A_q.shape
    Dm, H, Dh = B_Wq.shape
    M = B_mem0.shape[1]
    seg = int(B_seg_len)
    assert Bn == 1 and Dh == 128 and Dm == D and M == 8 and seg == 32
    assert S % (2 * seg) == 0 and S % 256 == 0 and D % 128 == 0 and D // 128 >= 2 and H % 16 == 0
    NG = D // 128
    fwd, inv = _dft_mats()

    any_spec = pl.BlockSpec(memory_space=pl.ANY)
    vmem_spec = pl.BlockSpec(memory_space=pltpu.VMEM)
    out = pl.pallas_call(
        functools.partial(_kernel, S=S, D=D, H=H, seg=seg, M=M),
        out_shape=jax.ShapeDtypeStruct((S, D), A_q.dtype),
        in_specs=[any_spec, any_spec, any_spec, vmem_spec, any_spec, vmem_spec, vmem_spec,
                  any_spec, any_spec, any_spec, any_spec, vmem_spec, vmem_spec, vmem_spec],
        out_specs=any_spec,
        scratch_shapes=[
            pltpu.VMEM((NG, S, 128), BF16),
            pltpu.VMEM((NG, S, 128), BF16),
            pltpu.VMEM((NG, S, 128), BF16),
            pltpu.VMEM((NG, 128, S), BF16),
            pltpu.VMEM((3, NSLOT, D * H // (2 * NG), 128), U32),
            pltpu.VMEM((3 * H, D // 2, 128), U32),
            pltpu.VMEM((NG, H * Dh // 2, 128), U32),
            pltpu.VMEM((NG, S, 128), BF16),
            pltpu.VMEM((S, 128), F32),
            pltpu.VMEM((S, D), BF16),
            pltpu.VMEM((1, D), F32),
            pltpu.VMEM((3 * H, S // seg * 8, 128), F32),
            pltpu.VMEM((S // seg * 4, 128), U32),
            pltpu.VMEM((S, 128), BF16),
            pltpu.VMEM((S // C, 3 * C, 128), F32),
            pltpu.VMEM((S // C, 3 * C, 128), F32),
            pltpu.VMEM((S // C, 2 * C, 128), F32),
            pltpu.VMEM((M, D), F32),
            pltpu.VMEM((H, 8, 128), F32),
            pltpu.VMEM((H, 24, 128), U32),
            pltpu.VMEM((48, D), F32),
            pltpu.SemaphoreType.DMA((7, NG)),
            pltpu.SemaphoreType.DMA((NG,)),
            pltpu.SemaphoreType.DMA(()),
        ],
        compiler_params=pltpu.CompilerParams(vmem_limit_bytes=120 * 1024 * 1024),
    )(
        A_q.reshape(S, D), A_k.reshape(S, D), A_v.reshape(S, D), A_shift_k.T, A_ssm_k,
        A_ssm_D, B_mem0.reshape(M, D),
        B_Wq.reshape(D * H, Dh), B_Wk.reshape(D * H, Dh), B_Wv.reshape(D * H, Dh),
        B_Wo.reshape(H * Dh, D), gate_w,
        jnp.asarray(fwd, BF16), jnp.asarray(inv, BF16),
    )
    return out.reshape(Bn, S, D)
```

```python
import functools

import jax
import jax.numpy as jnp
import numpy as np
import jax.experimental.pallas as pl
import jax.experimental.pallas.tpu as pltpu

F32 = jnp.float32
BF16 = jnp.bfloat16
U32 = jnp.uint32

NSLOT = 3
C = 128


def _dft_mats():
    f = np.arange(C, dtype=np.float64)[:, None] + 0.5
    t = np.arange(C, dtype=np.float64)[None, :]
    ang = 2.0 * np.pi * f * t / (2 * C)
    fwd = np.concatenate([np.cos(ang), -np.sin(ang)], axis=0)
    inv = np.concatenate([np.cos(ang).T, -np.sin(ang).T], axis=1) * (2.0 / (2 * C))
    return fwd.astype(np.float32), inv.astype(np.float32)


def _nt(a, b):
    return jax.lax.dot_general(a, b, (((1,), (1,)), ((), ())), preferred_element_type=F32)


def _nn(a, b):
    return jnp.dot(a, b, preferred_element_type=F32)


def _push(stack, x):
    n = 1
    while stack and stack[-1][0] == n:
        m, y = stack.pop()
        x, n = y + x, n + m
    stack.append((n, x))


def _total(stack):
    x = stack[-1][1]
    for _, y in reversed(stack[:-1]):
        x = y + x
    return x


def _kernel(q_hbm, k_hbm, v_hbm, shift_ref, ssmk_hbm, ssmd_ref, mem0_ref,
            wq_hbm, wk_hbm, wv_hbm, wo_hbm, gate_ref, f_ref, fi_ref,
            out_hbm,
            qbuf, kbuf, vbuf, sbuf, raw, wqkv, wo, abuf, gbuf, obuf,
            dskip, pre, xpre, kvbuf, asp, ksp, ysp, membuf, pendo, o32, pacc,
            sem_in, sem_wo, sem_out,
            *, S, D, H, seg, M):
    NG = D // 128
    NCH = S // C
    DCH = D // NG
    HP = H // 2
    CR = DCH * HP
    NSEG = S // seg
    PRE = NSEG * 8

    def in_copies(g):
        g = jnp.int32(g)
        sl = pl.ds(pl.multiple_of(g * 128, 128), 128)
        rows = pl.ds(pl.multiple_of(g * CR, CR), CR)
        cps = [pltpu.make_async_copy(k_hbm.at[:, sl], kbuf.at[g], sem_in.at[0, g]),
               pltpu.make_async_copy(v_hbm.at[:, sl], vbuf.at[g], sem_in.at[1, g]),
               pltpu.make_async_copy(ssmk_hbm.at[sl, :], sbuf.at[g], sem_in.at[2, g]),
               pltpu.make_async_copy(q_hbm.at[:, sl], qbuf.at[g], sem_in.at[3, g])]
        for i, w in enumerate((wq_hbm, wk_hbm, wv_hbm)):
            cps.append(pltpu.make_async_copy(
                w.bitcast(U32).at[rows, :], raw.at[i, jax.lax.rem(g, NSLOT)], sem_in.at[4 + i, g]))
        return cps

    def wo_copy(n):
        return pltpu.make_async_copy(
            wo_hbm.bitcast(U32).at[:, pl.ds(n * 128, 128)], wo.at[n], sem_wo.at[n])

    AHEAD = NSLOT - 1
    for g in range(AHEAD):
        for cp in in_copies(g):
            cp.start()

    def zero_pre(i, _):
        pre[i] = jnp.zeros((PRE, 128), F32)
        return 0

    jax.lax.fori_loop(0, 3 * H, zero_pre, 0)

    ks = shift_ref.shape[0]
    dskip[...] = ssmd_ref[...].astype(F32).reshape(1, D)
    fmat = f_ref[...]
    sgn = 1.0 - 2.0 * (jax.lax.broadcasted_iota(jnp.int32, (8, 128), 0) % 2).astype(F32)

    def repack(g, i, b):
        src = pl.ds(pl.multiple_of(b * 16 * HP, 16 * HP), 16 * HP)
        x = raw[i, jax.lax.rem(g, NSLOT), src, :].reshape(8, 2, HP // 8, 8, 128)
        dst = pl.ds(pl.multiple_of(g * (DCH // 2) + b * 8, 8), 8)
        for t in range(HP // 8):
            ev = jnp.transpose(x[:, 0, t], (1, 0, 2))
            od = jnp.transpose(x[:, 1, t], (1, 0, 2))
            for j in range(8):
                h = i * H + 2 * (8 * t + j)
                wqkv[h, dst, :] = (ev[j] & 0xFFFF) | (od[j] << 16)
                wqkv[h + 1, dst, :] = (ev[j] >> 16) | (od[j] & U32(0xFFFF0000))

    NSB = 8
    assert (DCH // 16) % NSB == 0 and (C // 8) % NSB == 0 and (3 * H) % NSB == 0

    def gather_pre(g):
        for sgi in range(0, NSEG, 2):
            xpre[sgi * 4:(sgi + 2) * 4, :] = pltpu.bitcast(jnp.concatenate(
                [qbuf[g, sgi * seg:sgi * seg + 8, :],
                 qbuf[g, (sgi + 1) * seg:(sgi + 1) * seg + 8, :]], axis=0), U32)

    def pre_tiles(g, sb, tts):
        krows = pl.ds(pl.multiple_of(g * 64, 64), 64)
        for tt in tts:
            idx = sb * (3 * H // NSB) + tt
            pre[idx] = pre[idx] + _nn(pltpu.bitcast(xpre[...], BF16),
                                        pltpu.bitcast(wqkv[idx, krows, :], BF16))

    def conv_group(g, _, with_pre=True):
        for cp in in_copies(g):
            cp.wait()

        @pl.when(g + AHEAD < NG)
        def _():
            for cp in in_copies(g + AHEAD):
                cp.start()

        @pl.when(g + AHEAD == NG)
        def _():
            for n in range(NG):
                wo_copy(n).start()

        lanes = pl.ds(pl.multiple_of(g * 128, 128), 128)
        tp = shift_ref[:, lanes].astype(F32)
        dvec = dskip[:, lanes]
        for j in range(NCH):
            cur = kbuf[g, j * C:(j + 1) * C, :].astype(F32)
            if j == 0:
                prev = jnp.zeros((16, 128), F32)
            else:
                prev = kbuf[g, j * C - 16:j * C, :].astype(F32)
            ext = jnp.concatenate([prev, cur], axis=0)
            acc = cur * tp[0:1, :]
            for u in range(1, ks):
                acc = acc + ext[16 - u:16 - u + C, :] * tp[u:u + 1, :]
            kv = (acc * vbuf[g, j * C:(j + 1) * C, :].astype(F32)).astype(BF16)
            kvbuf[j * C:(j + 1) * C, :] = kv
            asp[j] = _nn(fmat, kv)
            ksp[j] = _nt(fmat, sbuf[g, :, j * C:(j + 1) * C])

        if with_pre:
            gather_pre(g - 1)

        def super_block(sb, _):
            nf = C // 8 // NSB
            nt = 3 * H // NSB
            for fi in range(nf):
                if with_pre:
                    pre_tiles(g - 1, sb, range(fi * nt // nf, (fi + 1) * nt // nf))
                freq_block(sb * nf + fi)
            for b in range(DCH // 16 // NSB):
                for i in range(3):
                    repack(g, i, sb * (DCH // 16 // NSB) + b)
            return 0

        def freq_block(fb):
            rr = pl.ds(pl.multiple_of(fb * 8, 8), 8)
            ri = pl.ds(pl.multiple_of(C + fb * 8, 8), 8)
            prev_z = None
            IB = 4
            for i0 in range(0, NCH, IB):
                kc = {}
                acc = [[[], [], []] for _ in range(IB)]
                for j in range(i0 + IB):
                    ar, ai = asp[j, rr, :], asp[j, ri, :]
                    asum = ar + ai
                    for ii in range(IB):
                        m = i0 + ii - j
                        if m < 0:
                            continue
                        if m not in kc:
                            k_r, k_i = ksp[m, rr, :], ksp[m, ri, :]
                            kc[m] = (k_r, k_i - k_r, k_i + k_r)
                        kr, kdif, ksum = kc[m]
                        _push(acc[ii][0], kr * asum)
                        _push(acc[ii][1], ar * kdif)
                        _push(acc[ii][2], ai * ksum)
                acc = [[_total(x) for x in z] for z in acc]
                zr = [z[0] - z[2] for z in acc]
                zi = [z[0] + z[1] for z in acc]
                for ii in range(IB):
                    if prev_z is None:
                        yr, yi = zr[ii], zi[ii]
                    else:
                        yr = zr[ii] - sgn * prev_z[1]
                        yi = zi[ii] + sgn * prev_z[0]
                    prev_z = (zr[ii], zi[ii])
                    ysp[i0 + ii, rr, :] = yr
                    ysp[i0 + ii, ri, :] = yi

        jax.lax.fori_loop(0, NSB, super_block, 0)

        fimat = fi_ref[...]
        for j in range(NCH):
            y = _nn(fimat, ysp[j].astype(BF16)).astype(BF16).astype(F32)
            kv = kvbuf[j * C:(j + 1) * C, :].astype(F32)
            y = (y + (kv * dvec).astype(BF16).astype(F32)).astype(BF16).astype(F32)
            qv = qbuf[g, j * C:(j + 1) * C, :].astype(F32)
            abuf[g, j * C:(j + 1) * C, :] = (qv * y).astype(BF16)
        return 0

    conv_group(jnp.int32(0), 0, with_pre=False)
    jax.lax.fori_loop(1, NG, conv_group, 0)
    gather_pre(NG - 1)

    def last_pre(sb, _):
        pre_tiles(jnp.int32(NG - 1), sb, range(3 * H // NSB))
        return 0

    jax.lax.fori_loop(0, NSB, last_pre, 0)

    gw = jnp.broadcast_to(gate_ref[...].reshape(1, D), (128, D))
    RB = 256

    def gate_blk(i, _):
        rows = pl.ds(pl.multiple_of(i * RB, RB), RB)
        x = jnp.concatenate([qbuf[g, rows, :] for g in range(NG)], axis=1)
        z = _nt(x, gw)
        gbuf[rows, :] = jax.nn.sigmoid(z)
        return 0

    jax.lax.fori_loop(0, S // RB, gate_blk, 0)

    for n in range(NG):
        wo_copy(n).wait()

    membuf[...] = mem0_ref[...].astype(F32)
    L = M + seg
    scale = 128 ** -0.5
    row = jax.lax.broadcasted_iota(jnp.int32, (L, 48), 0)
    col = jax.lax.broadcasted_iota(jnp.int32, (L, 48), 1)
    mask = (col < L) & ((row < M) | (row >= col))

    LAG = 4
    HS = 16
    E0 = 4

    def step(u, even):
        r0 = pl.multiple_of(u * 2 * seg, 2 * seg)
        xs, nx = pl.multiple_of(r0 + (8 if even else seg + 8), 8), seg - 8
        prow = pl.ds(pl.multiple_of(u * 16 + (0 if even else 8), 8), 8)
        lhs = jnp.concatenate(
            [jnp.concatenate([membuf[:, g * 128:(g + 1) * 128],
                              qbuf[g, pl.ds(xs, nx), :].astype(F32)], axis=0)
             for g in range(NG)], axis=1).astype(BF16)

        rows_o = 32 if even else 48
        nb = rows_o - M
        b0 = pl.multiple_of(r0 if even else r0 + 24, 8)
        brow = pl.ds(b0, nb)
        qkv, es = {}, {}

        def proj(h):
            res = []
            for i in range(3):
                r = _nn(lhs, pltpu.bitcast(wqkv[i * H + h], BF16))
                full = jnp.concatenate(
                    [r[0:M], pre[i * H + h, prow, :], r[M:], jnp.zeros((8, 128), F32)], axis=0)
                res.append(full.astype(BF16))
            qkv[h] = res

        def scores(h):
            qh, kh, _ = qkv[h]
            s = _nt(qh, kh)[:L]
            s = jnp.where(mask, s, -1e9 / scale)
            mx = jnp.max(s, axis=1, keepdims=True)
            e = jnp.exp((s - mx) * scale)
            l = jnp.sum(e, axis=1, keepdims=True)
            e = jnp.concatenate([e, jnp.zeros((48 - L, 48), F32)], axis=0).astype(BF16)
            es[h] = (e, 1.0 / l)

        def attend(h):
            e, rl = es.pop(h)
            o = _nn(e, qkv.pop(h)[2])[:L] * rl
            if even:
                pendo[h] = o[32:40]
                o32[h, 0:16, :] = pltpu.bitcast(o[0:32].astype(BF16), U32)
            else:
                oo = jnp.concatenate([o[0:8], pendo[h], o[8:40]], axis=0)
                o32[h] = pltpu.bitcast(oo.astype(BF16), U32)

        def out_proj(n, h0, h1):
            ol = jnp.concatenate(
                [pltpu.bitcast(o32[h, 0:rows_o // 2, :], BF16) for h in range(h0, h1)], axis=1)
            return _nn(ol, pltpu.bitcast(wo[n, h0 * 64:h1 * 64, :], BF16))

        def early_out(ns):
            for n in ns:
                pacc[0:rows_o, n * 128:(n + 1) * 128] = out_proj(n, 0, HS)

        for t in range(H + 1 + LAG):
            if t < H:
                proj(t)
            if t == H:
                early_out(range(0, E0))
            if 0 <= t - 1 < H:
                scores(t - 1)
            if t == H:
                early_out(range(E0, NG))
            if 0 <= t - 1 - LAG < H:
                attend(t - 1 - LAG)

        gv = gbuf[brow, :]
        for n in range(NG):
            r = out_proj(n, HS, H) + pacc[0:rows_o, n * 128:(n + 1) * 128]
            r = r.astype(BF16).astype(F32)
            membuf[:, n * 128:(n + 1) * 128] = r[0:M]
            b = r[M:]
            a = abuf[n, brow, :].astype(F32)
            obuf[brow, n * 128:(n + 1) * 128] = (b + gv * (a - b)).astype(BF16)

    def double_step(u, _):
        step(u, True)
        step(u, False)
        rows = pl.ds(pl.multiple_of(u * 2 * seg, 2 * seg), 2 * seg)
        pltpu.make_async_copy(obuf.at[rows, :], out_hbm.at[rows, :], sem_out).start()
        return 0

    jax.lax.fori_loop(0, S // (2 * seg), double_step, 0)
    pltpu.make_async_copy(obuf, out_hbm, sem_out).wait()


@functools.partial(jax.jit, static_argnames=("B_seg_len",))
def pallas_gated_mix__ssm_conv_h3__memory_aug_recurrent_mem_tr__prompt_kernel(
    A_q: jax.Array,
    A_k: jax.Array,
    A_v: jax.Array,
    A_shift_k: jax.Array,
    A_ssm_k: jax.Array,
    A_ssm_D: jax.Array,
    B_x: jax.Array,
    B_mem0: jax.Array,
    B_Wq: jax.Array,
    B_Wk: jax.Array,
    B_Wv: jax.Array,
    B_Wo: jax.Array,
    B_seg_len,
    gate_w: jax.Array,
):
    del B_x
    Bn, S, D = A_q.shape
    Dm, H, Dh = B_Wq.shape
    M = B_mem0.shape[1]
    seg = int(B_seg_len)
    assert Bn == 1 and Dh == 128 and Dm == D and M == 8 and seg == 32
    assert S % (2 * seg) == 0 and S % 256 == 0 and D % 128 == 0 and D // 128 >= 2 and H % 16 == 0
    NG = D // 128
    fwd, inv = _dft_mats()

    any_spec = pl.BlockSpec(memory_space=pl.ANY)
    vmem_spec = pl.BlockSpec(memory_space=pltpu.VMEM)
    out = pl.pallas_call(
        functools.partial(_kernel, S=S, D=D, H=H, seg=seg, M=M),
        out_shape=jax.ShapeDtypeStruct((S, D), A_q.dtype),
        in_specs=[any_spec, any_spec, any_spec, vmem_spec, any_spec, vmem_spec, vmem_spec,
                  any_spec, any_spec, any_spec, any_spec, vmem_spec, vmem_spec, vmem_spec],
        out_specs=any_spec,
        scratch_shapes=[
            pltpu.VMEM((NG, S, 128), BF16),
            pltpu.VMEM((NG, S, 128), BF16),
            pltpu.VMEM((NG, S, 128), BF16),
            pltpu.VMEM((NG, 128, S), BF16),
            pltpu.VMEM((3, NSLOT, D * H // (2 * NG), 128), U32),
            pltpu.VMEM((3 * H, D // 2, 128), U32),
            pltpu.VMEM((NG, H * Dh // 2, 128), U32),
            pltpu.VMEM((NG, S, 128), BF16),
            pltpu.VMEM((S, 128), F32),
            pltpu.VMEM((S, D), BF16),
            pltpu.VMEM((1, D), F32),
            pltpu.VMEM((3 * H, S // seg * 8, 128), F32),
            pltpu.VMEM((S // seg * 4, 128), U32),
            pltpu.VMEM((S, 128), BF16),
            pltpu.VMEM((S // C, 2 * C, 128), F32),
            pltpu.VMEM((S // C, 2 * C, 128), F32),
            pltpu.VMEM((S // C, 2 * C, 128), F32),
            pltpu.VMEM((M, D), F32),
            pltpu.VMEM((H, 8, 128), F32),
            pltpu.VMEM((H, 24, 128), U32),
            pltpu.VMEM((48, D), F32),
            pltpu.SemaphoreType.DMA((7, NG)),
            pltpu.SemaphoreType.DMA((NG,)),
            pltpu.SemaphoreType.DMA(()),
        ],
        compiler_params=pltpu.CompilerParams(vmem_limit_bytes=120 * 1024 * 1024),
    )(
        A_q.reshape(S, D), A_k.reshape(S, D), A_v.reshape(S, D), A_shift_k.T, A_ssm_k,
        A_ssm_D, B_mem0.reshape(M, D),
        B_Wq.reshape(D * H, Dh), B_Wk.reshape(D * H, Dh), B_Wv.reshape(D * H, Dh),
        B_Wo.reshape(H * Dh, D), gate_w,
        jnp.asarray(fwd, BF16), jnp.asarray(inv, BF16),
    )
    return out.reshape(Bn, S, D)
```
